```python
import os as _os
_os.environ.setdefault("JAX_PLATFORMS", "cpu")
import jax
import jax.numpy as jnp

def _softmax(x, axis=-1):
    return jax.nn.softmax(x, axis=axis)
def _gelu(x):
    return jax.nn.gelu(x, approximate=True)
def _silu(x):
    return jax.nn.silu(x)
def _sigmoid(x):
    return jax.nn.sigmoid(x)
def _layernorm(x, axis=-1, eps=1e-5):
    m = jnp.mean(x, axis=axis, keepdims=True)
    v = jnp.var(x, axis=axis, keepdims=True)
    return (x - m) / jnp.sqrt(v + eps)
def _scatter_add(tgt, idx, src, axis=0):
    return tgt.at[idx].add(src)
def _segment_sum(src, seg, n):
    return jax.ops.segment_sum(src, seg, n)
class _Rng:
    def __init__(self, key):
        self._k = key
    def _next(self):
        self._k, sub = jax.random.split(self._k)
        return sub
    def normal(self, shape):
        return jax.random.normal(self._next(), shape, dtype=jnp.bfloat16)
    def randint(self, lo, hi, shape):
        return jax.random.randint(self._next(), shape, lo, hi, dtype=jnp.int32)
    def uniform(self, shape, lo=0.0, hi=1.0):
        return jax.random.uniform(self._next(), shape, jnp.bfloat16, lo, hi)
    def permutation(self, n):
        return jax.random.permutation(self._next(), n)


kernel_name = 'concat_heads__softmax_full_mha__ssm_conv_s5__prompt'

def setup_inputs():
    _rng = _Rng(jax.random.key(int.from_bytes(__import__("os").urandom(4), "little")))
    _w = (lambda a: (lambda t: t.astype(jnp.bfloat16) if jnp.issubdtype(t.dtype, jnp.floating) else t)(jnp.asarray(a)))
    def _A_setup():
        B, S, D = 1, 2048, 512
        return {
            "x": _w((lambda *s: _rng.normal(s) * 0.2)(B, S, D)),
            "wqkv": _w((lambda *s: _rng.normal(s) * 0.2)(D, 3 * D)),
            "wo": _w((lambda *s: _rng.normal(s) * 0.05)(D, D)),
        }
    _A_in = _A_setup()

    def _B_setup():
        B, S, D = 1, 2048, 512
        P = D
        Lambda_re = -0.5 * jnp.exp((lambda *s: _rng.normal(s) * 0.4)(P))
        Lambda_im = (lambda *s: _rng.normal(s) * 0.4)(P) * 1.0
        B_re = (lambda *s: _rng.normal(s) * 0.4)(P, D) * (D ** -0.5)
        B_im = (lambda *s: _rng.normal(s) * 0.4)(P, D) * (D ** -0.5)
        C_re = (lambda *s: _rng.normal(s) * 0.4)(D, P) * (P ** -0.5)
        C_im = (lambda *s: _rng.normal(s) * 0.4)(D, P) * (P ** -0.5)
        log_dt = (lambda *s: _rng.normal(s) * 0.4)(P) * 0.3 - 2.0
        Dskip = (lambda *s: _rng.normal(s) * 0.4)(D)
        return {
            "x": _w((lambda *s: _rng.normal(s) * 0.05)(B, S, D)),
            "Lambda_re": _w(Lambda_re),
            "Lambda_im": _w(Lambda_im),
            "B_re": _w(B_re),
            "B_im": _w(B_im),
            "C_re": _w(C_re),
            "C_im": _w(C_im),
            "log_dt": _w(log_dt),
            "Dskip": _w(Dskip),
        }
    _B_in = _B_setup()

    return {
        "A_x": _A_in["x"],
        "A_wqkv": _A_in["wqkv"],
        "A_wo": _A_in["wo"],
        "B_x": _B_in["x"],
        "B_Lambda_re": _B_in["Lambda_re"],
        "B_Lambda_im": _B_in["Lambda_im"],
        "B_B_re": _B_in["B_re"],
        "B_B_im": _B_in["B_im"],
        "B_C_re": _B_in["C_re"],
        "B_C_im": _B_in["C_im"],
        "B_log_dt": _B_in["log_dt"],
        "B_Dskip": _B_in["Dskip"],
    }

def reference(A_x, A_wqkv, A_wo, B_x, B_Lambda_re, B_Lambda_im, B_B_re, B_B_im, B_C_re, B_C_im, B_log_dt, B_Dskip):
    def _A_ref(x, wqkv, wo):
        B, S, D = x.shape
        H = 32; Dh = D // H
        qkv = (lambda x, *d: x.transpose(*d))((x @ wqkv).reshape(B, S, 3, H, Dh), 2, 0, 3, 1, 4)
        q, k, v = qkv[0], qkv[1], qkv[2]
        scale = Dh ** -0.5
        scores = jnp.einsum("bhqd,bhkd->bhqk", q, k) * scale
        p = _softmax(scores, axis=-1)
        o = jnp.einsum("bhqk,bhkd->bhqd", p, v)
        return (lambda x, *d: x.transpose(*d))(o, 0, 2, 1, 3).reshape(B, S, D) @ wo

    def _B_ref(x, Lambda_re, Lambda_im, B_re, B_im, C_re, C_im, log_dt, Dskip):
        Bsz, L, H = x.shape
        Lam = Lambda_re + 1j * Lambda_im
        Bmat = B_re + 1j * B_im
        Cmat = C_re + 1j * C_im
        dt = jnp.exp(log_dt)
        Lam_bar = jnp.exp(dt * Lam)
        B_bar = ((Lam_bar - 1.0) / Lam)[:, None] * Bmat
        Bu = jnp.einsum("bld,pd->blp", x + 0j, B_bar)
        h = jnp.zeros_like(Bu[:, 0, :])
        hs = []
        for t in range(L):
            h = Lam_bar[None, :] * h + Bu[:, t, :]
            hs.append(h)
        hseq = jnp.stack(hs, 1)
        y = 2.0 * jnp.einsum("blp,dp->bld", hseq, Cmat).real + x * Dskip[None, None, :]
        return y

    a = _A_ref(A_x, A_wqkv, A_wo)
    b = _B_ref(B_x, B_Lambda_re, B_Lambda_im, B_B_re, B_B_im, B_C_re, B_C_im, B_log_dt, B_Dskip)
    return jnp.concatenate([a, b], axis=-1)
```

```python
import math

import jax
import jax.numpy as jnp
import jax.experimental.pallas as pl
import jax.experimental.pallas.tpu as pltpu


F32 = jnp.float32
BF16 = jnp.bfloat16
U32 = jnp.uint32

SEQ = 2048
DM = 512
NHEAD = 32
DH = 16
TQ = 256
NQB = SEQ // TQ
UN = 4
PPB = NHEAD // UN
NPH = NQB * PPB
CK = 128
NC = SEQ // CK
NACC = 2
KG = 2
RB = 256
NRB = SEQ // RB
NCHUNK = 8
CLEN = SEQ // NCHUNK + 1
UROWS = NCHUNK * CLEN
SCAN_UNROLL = 4
NLT = DM // 128
QSCALE = (DH ** -0.5) * math.log2(math.e)
PK = False
PP = False
PV_ = False

_NT = (((1,), (1,)), ((), ()))
_TN = (((0,), (0,)), ((), ()))


def _dot(a, b, dims=(((1,), (0,)), ((), ()))):
    return jax.lax.dot_general(a, b, dims, preferred_element_type=F32)


def _red(x, op):
    r = x.shape[0]
    return op(x.reshape(r // (8 * NACC), 8 * NACC, x.shape[1]), axis=0)


def _pk(x):
    return pltpu.bitcast(x, U32)


def _upk(x):
    return pltpu.bitcast(x, BF16)


def _kernel(x_ref, wqkv_ref, wo_ref, xb_ref, lre_ref, lim_ref, bre_ref, bim_ref,
            cre_ref, cim_ref, ldt_ref, dsk_ref,
            o_ref,
            wt_s, qt_s, vt_s, kp_s, sA, sB, mA, mB, ot_s, ls_s,
            u_s, cp_s):
    j = pl.program_id(0)

    def rows16(ref, lead, head, c0, c1, packed):
        if packed:
            return _upk(ref[lead, pl.ds(pl.multiple_of(head * (DH // 2), DH // 2), DH // 2), c0:c1])
        return ref[lead, pl.ds(pl.multiple_of(head * DH, DH), DH), c0:c1]

    def get_w(g, t):
        jb = g // PPB
        head = (g % PPB) * UN + t
        q0 = jb * TQ
        if TQ >= RB:
            q = jnp.concatenate([rows16(qt_s, jb * (TQ // RB) + i, head, 0, RB, PV_) for i in range(TQ // RB)], axis=1)
        else:
            sub = RB // TQ
            q = rows16(qt_s, jb, head, 0, TQ, PV_)
        parts = [jnp.zeros((DH, TQ), BF16)] * KG
        parts[t % KG] = q
        return jnp.concatenate(parts, axis=0) if KG > 1 else q

    def qk_chunk(g, t, w, c, s_ref, macc):
        grp = (g % PPB) * (UN // KG) + t // KG
        if PK:
            k = _upk(kp_s[grp, c * CK // 2:(c + 1) * CK // 2, :])
        else:
            k = kp_s[grp, c * CK:(c + 1) * CK, :]
        s = _dot(k, w)
        s_ref[t, c * CK:(c + 1) * CK, :] = s
        r = _red(s, jnp.max)
        return r if macc is None else jnp.maximum(macc, r)

    def ex_chunk(m, t, c, s_ref, lacc):
        s = s_ref[t, c * CK:(c + 1) * CK, :].reshape(CK // 8, 8, TQ)
        p = jnp.exp2(s - m[None]).reshape(CK, TQ)
        r = _red(p, jnp.sum)
        return p.astype(BF16), (r if lacc is None else lacc + r)

    def pv_chunk(g, t, c, p, oacc):
        head = (g % PPB) * UN + t
        k0 = c * CK
        if CK <= RB:
            vt = rows16(vt_s, k0 // RB, head, k0 % RB, k0 % RB + CK, PV_)
        else:
            vt = jnp.concatenate([rows16(vt_s, k0 // RB + i, head, 0, RB, PV_) for i in range(CK // RB)], axis=1)
        o = _dot(vt, p)
        return o if oacc is None else oacc + o

    LEAD = 2

    def phase(ph, N_, C_, do_qk=True, do_pv=True):
        sN, mN = N_
        sC, mC = C_
        steps = [(t, c) for t in range(UN) for c in range(NC)]
        n = len(steps)
        ws, ms, laccs, ps = {}, {}, {}, {}
        macc = oacc = None

        def do_exp(i):
            t, c = steps[i]
            if c == 0:
                ms[t] = jnp.broadcast_to(mC[t], (8, TQ))
                laccs[t] = None
            ps[i], laccs[t] = ex_chunk(ms[t], t, c, sC, laccs[t])

        if do_pv:
            for i in range(min(LEAD, n)):
                do_exp(i)
        for i, (t, c) in enumerate(steps):
            if do_qk:
                if c == 0:
                    ws[t] = get_w(ph + 1, t)
                    macc = None
                macc = qk_chunk(ph + 1, t, ws[t], c, sN, macc)
                if c == NC - 1:
                    mN[t] = jnp.max(macc, axis=0, keepdims=True)
            if do_pv:
                if i + LEAD < n:
                    do_exp(i + LEAD)
                if c == 0:
                    oacc = None
                oacc = pv_chunk(ph, t, c, ps.pop(i), oacc)
                if c == NC - 1:
                    head = (ph % PPB) * UN + t
                    ot_s[head] = oacc
                    ls_s[head] = jnp.sum(laccs[t], axis=0, keepdims=True)

    A = (sA, mA)
    B = (sB, mB)

    @pl.when(j == 0)
    def _prologue():
        wt_s[0] = wqkv_ref[:, 0:DM].T
        wt_s[1] = wqkv_ref[:, 2 * DM:3 * DM].T

        def proj(i, carry):
            r0 = pl.multiple_of(i * RB, RB)
            xc = x_ref[pl.ds(r0, RB), :]
            qt = (_dot(wt_s[0], xc, _NT) * QSCALE).astype(BF16)
            vt = _dot(wt_s[1], xc, _NT).astype(BF16)
            if PV_:
                qt, vt = _pk(qt), _pk(vt)
            if TQ >= RB:
                qt_s[i] = qt
            else:
                for q in range(RB // TQ):
                    qt_s[i * (RB // TQ) + q] = qt[:, q * TQ:(q + 1) * TQ]
            vt_s[i] = vt
            k = _dot(xc, wqkv_ref[:, DM:2 * DM]).astype(BF16)
            if PK:
                k = _pk(k)
                r1 = pl.multiple_of(i * (RB // 2), RB // 2)
                for p in range(NHEAD // KG):
                    kp_s[p, pl.ds(r1, RB // 2), :] = k[:, DH * KG * p:DH * KG * (p + 1)]
            else:
                for p in range(NHEAD // KG):
                    kp_s[p, pl.ds(r0, RB), :] = k[:, DH * KG * p:DH * KG * (p + 1)]
            xb = xb_ref[pl.ds(r0, RB), :]
            ure = _dot(xb, bre_ref[...], _NT)
            uim = _dot(xb, bim_ref[...], _NT)
            for lt in range(NLT):
                u_s[lt, pl.ds(r0, RB), :] = ure[:, lt * 128:(lt + 1) * 128]
                u_s[NLT + lt, pl.ds(r0, RB), :] = uim[:, lt * 128:(lt + 1) * 128]
            return carry
        jax.lax.fori_loop(0, NRB, proj, 0)

        lam_re = lre_ref[...].astype(F32)
        lam_im = lim_ref[...].astype(F32)
        dt = jnp.exp(ldt_ref[...].astype(F32)).astype(BF16).astype(F32)
        mag = jnp.exp(dt * lam_re)
        ang = dt * lam_im
        lb_re = mag * jnp.cos(ang)
        lb_im = mag * jnp.sin(ang)
        den = lam_re * lam_re + lam_im * lam_im
        nre = lb_re - 1.0
        co_re = (nre * lam_re + lb_im * lam_im) / den
        co_im = (lb_im * lam_re - nre * lam_im) / den
        cre = cre_ref[...].astype(F32)
        cim = cim_ref[...].astype(F32)
        cp_s[:, 0:DM] = (2.0 * (cre * co_re - cim * co_im)).astype(BF16)
        cp_s[:, DM:2 * DM] = (-2.0 * (cre * co_im + cim * co_re)).astype(BF16)

        ar = [jnp.broadcast_to(lb_re[:, lt * 128:(lt + 1) * 128], (NCHUNK, 128)) for lt in range(NLT)]
        ai = [jnp.broadcast_to(lb_im[:, lt * 128:(lt + 1) * 128], (NCHUNK, 128)) for lt in range(NLT)]

        def scan_step(s, st, store):
            st = list(st)
            for lt in range(NLT):
                hr, hi = st[lt], st[NLT + lt]
                ur = u_s[lt, pl.ds(s, NCHUNK, stride=CLEN), :]
                ui = u_s[NLT + lt, pl.ds(s, NCHUNK, stride=CLEN), :]
                nr = ar[lt] * hr - ai[lt] * hi + ur
                ni = ar[lt] * hi + ai[lt] * hr + ui
                if store:
                    u_s[lt, pl.ds(s, NCHUNK, stride=CLEN), :] = nr
                    u_s[NLT + lt, pl.ds(s, NCHUNK, stride=CLEN), :] = ni
                st[lt], st[NLT + lt] = nr, ni
            return tuple(st)

        def scan(st, store):
            def body(i, st):
                for k in range(SCAN_UNROLL):
                    st = scan_step(i * SCAN_UNROLL + k, st, store)
                return st
            nfull = CLEN // SCAN_UNROLL
            st = jax.lax.fori_loop(0, nfull, body, st)
            for s in range(nfull * SCAN_UNROLL, CLEN):
                st = scan_step(s, st, store)
            return st

        for lt in range(2 * NLT):
            u_s[lt, SEQ:UROWS, :] = jnp.zeros((UROWS - SEQ, 128), F32)
        zero = tuple(jnp.zeros((NCHUNK, 128), F32) for _ in range(2 * NLT))
        ends = scan(zero, False)
        row = jax.lax.broadcasted_iota(jnp.int32, (NCHUNK, 128), 0)
        init = []
        for lt in range(NLT):
            br, bi = ar[lt], ai[lt]
            pr = pi = None
            e = CLEN
            while e:
                if e & 1:
                    pr, pi = (br, bi) if pr is None else (pr * br - pi * bi, pr * bi + pi * br)
                e >>= 1
                if e:
                    br, bi = br * br - bi * bi, 2.0 * br * bi
            hr = jnp.where(row >= 1, pltpu.roll(ends[lt], 1, 0), 0.0)
            hi = jnp.where(row >= 1, pltpu.roll(ends[NLT + lt], 1, 0), 0.0)
            sh = 1
            while sh < NCHUNK:
                sr = jnp.where(row >= sh, pltpu.roll(hr, sh, 0), 0.0)
                si = jnp.where(row >= sh, pltpu.roll(hi, sh, 0), 0.0)
                hr, hi = hr + pr * sr - pi * si, hi + pr * si + pi * sr
                pr, pi = pr * pr - pi * pi, 2.0 * pr * pi
                sh *= 2
            init.append((hr, hi))
        init = tuple(h[0] for h in init) + tuple(h[1] for h in init)
        scan(init, True)

    QPS = RB // TQ if TQ <= RB else 1
    assert TQ <= RB
    PPS = PPB * QPS

    @pl.when(j == 0)
    def _fill0():
        phase(-1, A, B, do_pv=False)

    def finish_qblock(sub):
        o = (ot_s[...] * (1.0 / ls_s[...])).reshape(DM, TQ).astype(BF16)
        o_ref[pl.ds(pl.multiple_of(sub * TQ, TQ), TQ), 0:DM] = _dot(o, wo_ref[...], _TN)

    def one_phase(i, carry):
        ph = j * PPS + i

        @pl.when(i % 2 == 0)
        def _even():
            phase(ph, B, A)

        @pl.when(i % 2 == 1)
        def _odd():
            phase(ph, A, B)

        if QPS > 1:
            @pl.when(jnp.logical_and(i % PPB == PPB - 1, i < PPS - 1))
            def _fin():
                finish_qblock(i // PPB)
        return carry

    nph = jnp.where(j == NRB - 1, PPS - 1, PPS)
    jax.lax.fori_loop(0, nph, one_phase, 0)

    @pl.when(j == NRB - 1)
    def _tail():
        phase(NPH - 1, A, B, do_qk=False)

    finish_qblock(QPS - 1)
    r0 = pl.multiple_of(j * RB, RB)
    g = jnp.concatenate([u_s[lt, pl.ds(r0, RB), :] for lt in range(2 * NLT)], axis=1).astype(BF16)
    y = _dot(g, cp_s[...], _NT)
    o_ref[:, DM:2 * DM] = y + xb_ref[pl.ds(r0, RB), :].astype(F32) * dsk_ref[...].astype(F32)


@jax.jit
def pallas_concat_heads__softmax_full_mha__ssm_conv_s5__prompt_kernel(
    A_x, A_wqkv, A_wo, B_x, B_Lambda_re, B_Lambda_im, B_B_re, B_B_im, B_C_re, B_C_im,
    B_log_dt, B_Dskip,
):
    def full(shape):
        return pl.BlockSpec(shape, lambda j: (0,) * len(shape))

    vec = lambda a: a.reshape(1, DM)
    args = (A_x.reshape(SEQ, DM), A_wqkv, A_wo, B_x.reshape(SEQ, DM), vec(B_Lambda_re),
            vec(B_Lambda_im), B_B_re, B_B_im, B_C_re, B_C_im, vec(B_log_dt), vec(B_Dskip))
    pdt = lambda packed: U32 if packed else BF16
    pn = lambda n, packed: n // 2 if packed else n
    scratch = [
        pltpu.VMEM((2, DM, DM), BF16),
        pltpu.VMEM((NQB, pn(DM, PV_), TQ), pdt(PV_)),
        pltpu.VMEM((NRB, pn(DM, PV_), RB), pdt(PV_)),
        pltpu.VMEM((NHEAD // KG, pn(SEQ, PK), DH * KG), pdt(PK)),
        pltpu.VMEM((UN, SEQ, TQ), F32),
        pltpu.VMEM((UN, SEQ, TQ), F32),
        pltpu.VMEM((UN, 1, TQ), F32),
        pltpu.VMEM((UN, 1, TQ), F32),
        pltpu.VMEM((NHEAD, DH, TQ), F32),
        pltpu.VMEM((NHEAD, 1, TQ), F32),
        pltpu.VMEM((2 * NLT, UROWS, 128), F32),
        pltpu.VMEM((DM, 2 * DM), BF16),
    ]
    out = pl.pallas_call(
        _kernel,
        grid=(NRB,),
        in_specs=[full(a.shape) for a in args],
        out_specs=pl.BlockSpec((RB, 2 * DM), lambda j: (j, 0)),
        out_shape=jax.ShapeDtypeStruct((SEQ, 2 * DM), F32),
        scratch_shapes=scratch,
        compiler_params=pltpu.CompilerParams(
            dimension_semantics=("arbitrary",),
            vmem_limit_bytes=110 * 1024 * 1024),
    )(*args)
    return out.reshape(1, SEQ, 2 * DM)
```

```python
import math

import jax
import jax.numpy as jnp
import jax.experimental.pallas as pl
import jax.experimental.pallas.tpu as pltpu

F32 = jnp.float32
BF16 = jnp.bfloat16

SEQ = 2048
DM = 512
NHEAD = 32
DH = 16
TQ = 256
NQB = SEQ // TQ
UN = 8
PPB = NHEAD // UN
NPH = NQB * PPB
CK = 128
NC = SEQ // CK
NACC = 2
KG = 4
LEAD = 2
VR = 16
OFF = 3
LA = 3
LB = 6
LAG = 8
PU = 2
NCHUNK = 8
CLEN = SEQ // NCHUNK + 1
UROWS = NCHUNK * CLEN
NLT = DM // 128
QSCALE = (DH ** -0.5) * math.log2(math.e)

_NN = (((1,), (0,)), ((), ()))
_NT = (((1,), (1,)), ((), ()))
_TN = (((0,), (0,)), ((), ()))

S_WQ, S_WK, S_WV, S_BRE, S_BIM, S_CRE, S_CIM, S_WO, S_X0 = range(9)
S_XB0 = S_X0 + NQB
S_OUT = S_XB0 + NQB
NSEM = S_OUT + 4


def _dot(a, b, dims=_NN):
    return jax.lax.dot_general(a, b, dims, preferred_element_type=F32)


def _red(x, op):
    r = x.shape[0]
    return op(x.reshape(r // (8 * NACC), 8 * NACC, x.shape[1]), axis=0)


def _zero_of(v):
    i = v.astype(jnp.int32)
    i = jax.lax.shift_right_logical(jax.lax.shift_right_logical(i, 31), 1)
    return i.astype(F32)


def _cmul(ar, ai, br, bi):
    return ar * br - ai * bi, ar * bi + ai * br


def _kernel(x_hbm, wqkv_hbm, wo_hbm, xb_hbm, lre_ref, lim_ref, bre_hbm, bim_hbm,
            cre_hbm, cim_hbm, ldt_ref, dsk_ref,
            o_hbm,
            x_s, w_s, wo_s, xb_s, bre_s, bim_s, cre_s, cim_s, o_s, sems,
            wt_s, qt_s, vt_s, kp_s, sA, sB, mA, mB, ot_s, ls_s, u_s, cp_s, kf_s, qf_s, par_s):
    j = pl.program_id(0)

    def rows_copy(src, dst, i, sem0):
        rows = pl.ds(pl.multiple_of(i * TQ, TQ), TQ)
        return pltpu.make_async_copy(src.at[rows], dst.at[rows], sems.at[sem0 + i])

    x_copy = lambda i: rows_copy(x_hbm, x_s, i, S_X0)
    xb_copy = lambda i: rows_copy(xb_hbm, xb_s, i, S_XB0)

    whole = {
        S_WQ: (wqkv_hbm.at[:, 0:DM], w_s.at[0]), S_WK: (wqkv_hbm.at[:, DM:2 * DM], w_s.at[1]),
        S_WV: (wqkv_hbm.at[:, 2 * DM:3 * DM], w_s.at[2]),
        S_BRE: (bre_hbm, bre_s), S_BIM: (bim_hbm, bim_s),
        S_CRE: (cre_hbm, cre_s), S_CIM: (cim_hbm, cim_s), S_WO: (wo_hbm, wo_s),
    }

    def copy(k):
        src, dst = whole[k]
        return pltpu.make_async_copy(src, dst, sems.at[k])

    def out_copy(step, half):
        slot = step % 2
        rows = pl.ds(pl.multiple_of(step * TQ, TQ), TQ)
        cols = pl.ds(half * DM, DM)
        return pltpu.make_async_copy(o_s.at[slot, :, cols], o_hbm.at[rows, cols],
                                     sems.at[S_OUT + 2 * slot + half])

    def head_rows(head):
        return pl.ds(pl.multiple_of(head * DH, DH), DH)

    def get_w(g, t):
        q = qt_s[g // PPB, head_rows((g % PPB) * UN + t), :]

        def pad(q):
            parts = [jnp.zeros((DH, TQ), BF16)] * KG
            parts[t % KG] = q
            return jnp.concatenate(parts, axis=0)

        w0 = pad(q)

        def make(z):
            if z is None:
                return w0
            zz = jnp.concatenate([z] * (TQ // 128), axis=1)[None]
            qz = q.astype(F32).reshape(DH // 8, 8, TQ) + zz
            return pad(qz.reshape(DH, TQ).astype(BF16))
        return make

    def qk_chunk(g, t, w, c, s_ref, macc, nrows):
        grp = (g % PPB) * (UN // KG) + t // KG
        s = _dot(kp_s[grp, c * CK:c * CK + nrows, :], w)
        s_ref[t, c * CK:c * CK + nrows, :] = s
        if nrows == CK:
            r = _red(s, jnp.max)
        else:
            r = jnp.max(s.reshape(nrows // VR, VR, TQ), axis=0)
        return r if macc is None else jnp.maximum(macc, r)

    def qk_vpu(g, t, c, s_ref, zin):
        kf = kf_s[g % PPB, c * VR:(c + 1) * VR, :]
        if zin is not None:
            kf = (kf.reshape(VR // 8, 8, 128) + zin[None]).reshape(VR, 128)
        acc = [[None] * (TQ // 128) for _ in range(VR // 8)]
        for d in range(DH):
            col = t * DH + d
            qb = [jnp.broadcast_to(qf_s[g, col:col + 1, qt * 128:(qt + 1) * 128], (8, 128))
                  for qt in range(TQ // 128)]
            for kg in range(VR // 8):
                kb = jnp.broadcast_to(kf[8 * kg:8 * kg + 8, col:col + 1], (8, 128))
                for qt in range(TQ // 128):
                    p = kb * qb[qt]
                    acc[kg][qt] = p if acc[kg][qt] is None else acc[kg][qt] + p
        s = jnp.concatenate([jnp.concatenate(a, axis=1) for a in acc], axis=0)
        s_ref[t, (c + 1) * CK - VR:(c + 1) * CK, :] = s
        return s

    def ex_chunk(m, t, c, s_ref, lacc):
        s = s_ref[t, c * CK:(c + 1) * CK, :].reshape(CK // 8, 8, TQ)
        p = jnp.exp2(s - m[None]).reshape(CK, TQ)
        r = _red(p, jnp.sum)
        return p.astype(BF16), (r if lacc is None else lacc + r)

    def pv_chunk(g, t, c, p, oacc, z):
        k0 = c * CK
        vt = vt_s[k0 // TQ, head_rows((g % PPB) * UN + t), k0 % TQ:k0 % TQ + CK]
        if z is not None:
            vt = (vt.astype(F32).reshape(DH // 8, 8, CK) + z[None]).reshape(DH, CK).astype(BF16)
        o = _dot(vt, p)
        return o if oacc is None else oacc + o

    def phase(ph, N_, C_, do_qk=True, do_pv=True, pre_qk=None, side=None):
        sN, mN = N_
        sC, mC = C_
        steps = [(t, c) for t in range(UN) for c in range(NC)]
        n = len(steps)
        ws, ms, laccs, ps = {}, {}, {}, {}
        macc = oacc = None
        hist = []
        pv_dep = {}

        def do_exp(i):
            t, c = steps[i]
            if c == 0:
                ms[t] = jnp.broadcast_to(mC[t], (8, TQ))
                laccs[t] = None
            ps[i], laccs[t] = ex_chunk(ms[t], t, c, sC, laccs[t])

        if do_pv:
            for i in range(min(LEAD, n)):
                do_exp(i)
        for i, (t, c) in enumerate(steps):
            if do_qk:
                if c == 0:
                    ws[t] = get_w(ph + 1, t)
                    macc = None
                z = pre_qk(i, hist) if pre_qk is not None else None
                off = do_pv and OFF > 0 and i % OFF == OFF - 1
                macc = qk_chunk(ph + 1, t, ws[t](z), c, sN, macc, CK - VR if off else CK)
                hist.append(macc[0:8, 0:128])
                if off:
                    zin = _zero_of(hist[i - LA]) if i >= LA else None
                    sv = qk_vpu(ph + 1, t, c, sN, zin)
                    macc = jnp.maximum(macc, sv)
                    pv_dep[i + LB] = _zero_of(sv[0:8, 0:128] + sv[8:16, 128:256])
                if c == NC - 1:
                    mN[t] = jnp.max(macc, axis=0, keepdims=True)
            if side is not None:
                side(i)
            if do_pv:
                if i + LEAD < n:
                    do_exp(i + LEAD)
                if c == 0:
                    oacc = None
                oacc = pv_chunk(ph, t, c, ps.pop(i), oacc, pv_dep.get(i))
                if c == NC - 1:
                    head = (ph % PPB) * UN + t
                    ot_s[head] = oacc
                    ls_s[head] = jnp.sum(laccs[t], axis=0, keepdims=True)

    A = (sA, mA)
    B = (sB, mB)

    def ssm_params():
        row1 = lambda ref: ref[...].astype(F32).reshape(1, DM)
        lam_re = row1(lre_ref)
        lam_im = row1(lim_ref)
        dt = jnp.exp(row1(ldt_ref)).astype(BF16).astype(F32)
        mag = jnp.exp(dt * lam_re)
        ang = dt * lam_im
        lb_re = mag * jnp.cos(ang)
        lb_im = mag * jnp.sin(ang)
        den = lam_re * lam_re + lam_im * lam_im
        nre = lb_re - 1.0
        par_s[0] = lb_re
        par_s[1] = lb_im
        par_s[2] = (nre * lam_re + lb_im * lam_im) / den
        par_s[3] = (lb_im * lam_re - nre * lam_im) / den

    def c_rows(r0, r1):
        co_re, co_im = par_s[2], par_s[3]
        cre = cre_s[r0:r1, :].astype(F32)
        cim = cim_s[r0:r1, :].astype(F32)
        a = 2.0 * (cre * co_re - cim * co_im)
        b = -2.0 * (cre * co_im + cim * co_re)
        cp_s[r0:r1, 0:DM] = a.astype(BF16)
        cp_s[r0:r1, DM:2 * DM] = b.astype(BF16)
        return a[0:8, 0:128]

    def scan_step(s, st, ar, ai, store):
        st = list(st)
        for lt in range(NLT):
            hr, hi = st[lt], st[NLT + lt]
            ur = u_s[lt, pl.ds(s, NCHUNK, stride=CLEN), :]
            ui = u_s[NLT + lt, pl.ds(s, NCHUNK, stride=CLEN), :]
            nr = ar[lt] * hr - ai[lt] * hi + ur
            ni = ar[lt] * hi + ai[lt] * hr + ui
            if store:
                u_s[lt, pl.ds(s, NCHUNK, stride=CLEN), :] = nr
                u_s[NLT + lt, pl.ds(s, NCHUNK, stride=CLEN), :] = ni
            st[lt], st[NLT + lt] = nr, ni
        return tuple(st)

    def chunk_carry(ends, ar, ai):
        row = jax.lax.broadcasted_iota(jnp.int32, (NCHUNK, 128), 0)
        init = []
        for lt in range(NLT):
            br, bi = ar[lt], ai[lt]
            pr = pi = None
            e = CLEN
            while e:
                if e & 1:
                    pr, pi = (br, bi) if pr is None else _cmul(pr, pi, br, bi)
                e >>= 1
                if e:
                    br, bi = _cmul(br, bi, br, bi)
            hr = jnp.where(row >= 1, pltpu.roll(ends[lt], 1, 0), 0.0)
            hi = jnp.where(row >= 1, pltpu.roll(ends[NLT + lt], 1, 0), 0.0)
            sh = 1
            while sh < NCHUNK:
                sr = jnp.where(row >= sh, pltpu.roll(hr, sh, 0), 0.0)
                si = jnp.where(row >= sh, pltpu.roll(hi, sh, 0), 0.0)
                dr, di = _cmul(pr, pi, sr, si)
                hr, hi = hr + dr, hi + di
                pr, pi = _cmul(pr, pi, pr, pi)
                sh *= 2
            init.append((hr, hi))
        return tuple(h[0] for h in init) + tuple(h[1] for h in init)

    class PacedScan:
        def __init__(self, nslices):
            lb_re, lb_im = par_s[0], par_s[1]
            tile = lambda v, lt: jnp.broadcast_to(v[:, lt * 128:(lt + 1) * 128], (NCHUNK, 128))
            self.ar = [tile(lb_re, lt) for lt in range(NLT)]
            self.ai = [tile(lb_im, lt) for lt in range(NLT)]
            self.st = tuple(jnp.zeros((NCHUNK, 128), F32) for _ in range(2 * NLT))
            self.items = [(False, s) for s in range(CLEN)] + [None] + [(True, s) for s in range(CLEN)]
            self.n = nslices
            self.crows = {(k * nslices) // (DM // 32): k for k in range(DM // 32)}

        def __call__(self, i, hist):
            lo = (i * len(self.items)) // self.n
            hi = ((i + 1) * len(self.items)) // self.n
            if i >= LAG:
                zin = _zero_of(hist[i - LAG])
                self.st = tuple(h + zin for h in self.st[:NLT]) + tuple(self.st[NLT:])
            for it in self.items[lo:hi]:
                if it is None:
                    self.st = chunk_carry(self.st, self.ar, self.ai)
                else:
                    self.st = scan_step(it[1], self.st, self.ar, self.ai, it[0])
            dep = (self.st[0] + self.st[1]) + (self.st[2] + self.st[3])
            if i in self.crows:
                k = self.crows[i]
                dep = dep + c_rows(32 * k, 32 * (k + 1))
            return _zero_of(dep)

    def proj_ssm_block(i):
        r0 = pl.multiple_of(i * TQ, TQ)
        xb = xb_s[pl.ds(r0, TQ), :]
        ure = _dot(xb, bre_s[...], _NT)
        uim = _dot(xb, bim_s[...], _NT)
        for lt in range(NLT):
            u_s[lt, pl.ds(r0, TQ), :] = ure[:, lt * 128:(lt + 1) * 128]
            u_s[NLT + lt, pl.ds(r0, TQ), :] = uim[:, lt * 128:(lt + 1) * 128]

    def proj_attn_block(i):
        r0 = pl.multiple_of(i * TQ, TQ)
        xc = x_s[pl.ds(r0, TQ), :]
        qt = (_dot(wt_s[0], xc, _NT) * QSCALE).astype(BF16)
        qt_s[i] = qt
        for hq in range(PPB):
            qf_s[i * PPB + hq] = qt[hq * UN * DH:(hq + 1) * UN * DH, :].astype(F32)
        vt_s[i] = _dot(wt_s[1], xc, _NT).astype(BF16)
        k = _dot(xc, w_s[1]).astype(BF16)
        for p in range(NHEAD // KG):
            kp_s[p, pl.ds(r0, TQ), :] = k[:, DH * KG * p:DH * KG * (p + 1)]
        for cc in range(TQ // CK):
            kr = k[(cc + 1) * CK - VR:(cc + 1) * CK, :].astype(F32)
            row = pl.multiple_of((i * (TQ // CK) + cc) * VR, VR)
            for lt in range(NLT):
                kf_s[lt, pl.ds(row, VR), :] = kr[:, lt * 128:(lt + 1) * 128]

    NPAIR = NQB // PU

    @pl.when(j == 0)
    def _prologue():
        copy(S_BRE).start()
        copy(S_BIM).start()
        for u in range(PU):
            xb_copy(u).start()
        ssm_params()
        for lt in range(2 * NLT):
            u_s[lt, SEQ:UROWS, :] = jnp.zeros((UROWS - SEQ, 128), F32)
        copy(S_BRE).wait()
        copy(S_BIM).wait()

        def proj_ssm(i, carry):
            for u in range(PU):
                xb_copy(i * PU + u).wait()

            @pl.when(i == 0)
            def _():
                for r in range(PU, NQB):
                    xb_copy(r).start()

            @pl.when(i == 1)
            def _():
                for k in (S_WQ, S_WV, S_WK):
                    copy(k).start()
                for r in range(NQB):
                    x_copy(r).start()

            for u in range(PU):
                proj_ssm_block(i * PU + u)
            return carry
        jax.lax.fori_loop(0, NPAIR - 1, proj_ssm, 0)

        for u in range(PU):
            xb_copy(NQB - PU + u).wait()
        copy(S_WQ).wait()
        copy(S_WV).wait()
        for k in (S_CRE, S_CIM, S_WO):
            copy(k).start()
        for u in range(PU):
            proj_ssm_block(NQB - PU + u)
            wt_s[u] = w_s[2 * u].T
        copy(S_WK).wait()

        def proj_attn(i, carry):
            for u in range(PU):
                x_copy(i * PU + u).wait()
            for u in range(PU):
                proj_attn_block(i * PU + u)
            return carry
        jax.lax.fori_loop(0, NPAIR, proj_attn, 0)

        for k in (S_CRE, S_CIM, S_WO):
            copy(k).wait()

    @pl.when(j == 0)
    def _fill():
        phase(-1, A, B, do_pv=False, pre_qk=PacedScan(UN * NC))

    def one_phase(i, carry):
        ph = j * PPB + i

        @pl.when(i % 2 == 0)
        def _even():
            phase(ph, B, A)

        @pl.when(i % 2 == 1)
        def _odd():
            phase(ph, A, B)
        return carry

    nph = jnp.where(j == NQB - 1, PPB - 1, PPB)
    jax.lax.fori_loop(0, nph, one_phase, 0)

    slot = j % 2

    @pl.when(j >= 2)
    def _free_slot():
        out_copy(j - 2, 0).wait()
        out_copy(j - 2, 1).wait()

    def ssm_out():
        r0 = pl.multiple_of(j * TQ, TQ)
        g = jnp.concatenate([u_s[lt, pl.ds(r0, TQ), :] for lt in range(2 * NLT)], axis=1).astype(BF16)
        y = _dot(g, cp_s[...], _NT)
        d = dsk_ref[...].astype(F32).reshape(1, DM)
        o_s[slot, :, DM:2 * DM] = y + xb_s[pl.ds(r0, TQ), :].astype(F32) * d

    def attn_out():
        o = (ot_s[...] * (1.0 / ls_s[...])).reshape(DM, TQ).astype(BF16)
        o_s[slot, :, 0:DM] = _dot(o, wo_s[...], _TN)

    class SsmOutPieces:
        def __init__(self, nsteps):
            self.r0 = (NQB - 1) * TQ
            self.npieces = NLT * 2 * NLT
            self.at = {(p * nsteps) // self.npieces: p for p in range(self.npieces)}
            self.acc = None

        def __call__(self, i):
            if i not in self.at:
                return
            n, k = divmod(self.at[i], 2 * NLT)
            g = u_s[k, self.r0:self.r0 + TQ, :].astype(BF16)
            part = _dot(g, cp_s[n * 128:(n + 1) * 128, k * 128:(k + 1) * 128], _NT)
            self.acc = part if k == 0 else self.acc + part
            if k == 2 * NLT - 1:
                d = dsk_ref[...].astype(F32).reshape(1, DM)[:, n * 128:(n + 1) * 128]
                xb = xb_s[self.r0:self.r0 + TQ, n * 128:(n + 1) * 128].astype(F32)
                o_s[(NQB - 1) % 2, :, DM + n * 128:DM + (n + 1) * 128] = self.acc + xb * d

    @pl.when(j < NQB - 1)
    def _notlast():
        ssm_out()
        attn_out()
        out_copy(j, 0).start()
        out_copy(j, 1).start()

    @pl.when(j == NQB - 1)
    def _last():
        phase(NPH - 1, A, B, do_qk=False, side=SsmOutPieces(UN * NC))
        out_copy(j, 1).start()

    @pl.when(j == NQB - 1)
    def _last2():
        attn_out()
        out_copy(j, 0).start()
        out_copy(j - 1, 0).wait()
        out_copy(j - 1, 1).wait()
        out_copy(j, 1).wait()
        out_copy(j, 0).wait()


@jax.jit
def pallas_concat_heads__softmax_full_mha__ssm_conv_s5__prompt_kernel(
    A_x, A_wqkv, A_wo, B_x, B_Lambda_re, B_Lambda_im, B_B_re, B_B_im, B_C_re, B_C_im,
    B_log_dt, B_Dskip,
):
    hbm = pl.BlockSpec(memory_space=pl.ANY)
    vec = pl.BlockSpec((DM,), lambda j: (0,))
    args = (A_x.reshape(SEQ, DM), A_wqkv, A_wo, B_x.reshape(SEQ, DM), B_Lambda_re,
            B_Lambda_im, B_B_re, B_B_im, B_C_re, B_C_im, B_log_dt, B_Dskip)
    in_specs = [hbm, hbm, hbm, hbm, vec, vec, hbm, hbm, hbm, hbm, vec, vec]
    scratch = [
        pltpu.VMEM((SEQ, DM), BF16),
        pltpu.VMEM((3, DM, DM), BF16),
        pltpu.VMEM((DM, DM), BF16),
        pltpu.VMEM((SEQ, DM), BF16),
        pltpu.VMEM((DM, DM), BF16),
        pltpu.VMEM((DM, DM), BF16),
        pltpu.VMEM((DM, DM), BF16),
        pltpu.VMEM((DM, DM), BF16),
        pltpu.VMEM((2, TQ, 2 * DM), F32),
        pltpu.SemaphoreType.DMA((NSEM,)),
        pltpu.VMEM((2, DM, DM), BF16),
        pltpu.VMEM((NQB, DM, TQ), BF16),
        pltpu.VMEM((NQB, DM, TQ), BF16),
        pltpu.VMEM((NHEAD // KG, SEQ, DH * KG), BF16),
        pltpu.VMEM((UN, SEQ, TQ), F32),
        pltpu.VMEM((UN, SEQ, TQ), F32),
        pltpu.VMEM((UN, 1, TQ), F32),
        pltpu.VMEM((UN, 1, TQ), F32),
        pltpu.VMEM((NHEAD, DH, TQ), F32),
        pltpu.VMEM((NHEAD, 1, TQ), F32),
        pltpu.VMEM((2 * NLT, UROWS, 128), F32),
        pltpu.VMEM((DM, 2 * DM), BF16),
        pltpu.VMEM((NLT, NC * VR, 128), F32),
        pltpu.VMEM((NPH, UN * DH, TQ), F32),
        pltpu.VMEM((4, 1, DM), F32),
    ]
    out = pl.pallas_call(
        _kernel,
        grid=(NQB,),
        in_specs=in_specs,
        out_specs=pl.BlockSpec(memory_space=pl.ANY),
        out_shape=jax.ShapeDtypeStruct((SEQ, 2 * DM), F32),
        scratch_shapes=scratch,
        compiler_params=pltpu.CompilerParams(
            dimension_semantics=("arbitrary",),
            vmem_limit_bytes=110 * 1024 * 1024),
    )(*args)
    return out.reshape(1, SEQ, 2 * DM)
```

```python
import math

import jax
import jax.numpy as jnp
import jax.experimental.pallas as pl
import jax.experimental.pallas.tpu as pltpu

F32 = jnp.float32
BF16 = jnp.bfloat16

SEQ = 2048
DM = 512
NHEAD = 32
DH = 16
TQ = 256
NQB = SEQ // TQ
UN = 8
PPB = NHEAD // UN
NPH = NQB * PPB
CK = 128
NC = SEQ // CK
NACC = 2
KG = 4
LEAD = 2
VR = 16
OFFC = (1, 3, 6, 8, 11, 13)
LA = 3
LB = 7
LAG = 8
PU = 2
NCHUNK = 8
CLEN = SEQ // NCHUNK + 1
UROWS = NCHUNK * CLEN
NLT = DM // 128
QSCALE = (DH ** -0.5) * math.log2(math.e)

_NN = (((1,), (0,)), ((), ()))
_NT = (((1,), (1,)), ((), ()))
_TN = (((0,), (0,)), ((), ()))

S_WQ, S_WK, S_WV, S_BRE, S_BIM, S_CRE, S_CIM, S_WO, S_X0 = range(9)
S_XB0 = S_X0 + NQB
S_OUT = S_XB0 + NQB
NSEM = S_OUT + 4


def _dot(a, b, dims=_NN):
    return jax.lax.dot_general(a, b, dims, preferred_element_type=F32)


def _red(x, op):
    r = x.shape[0]
    return op(x.reshape(r // (8 * NACC), 8 * NACC, x.shape[1]), axis=0)


def _zero_of(v):
    i = v.astype(jnp.int32)
    i = jax.lax.shift_right_logical(jax.lax.shift_right_logical(i, 31), 1)
    return i.astype(F32)


def _cmul(ar, ai, br, bi):
    return ar * br - ai * bi, ar * bi + ai * br


def _kernel(x_hbm, wqkv_hbm, wo_hbm, xb_hbm, lre_ref, lim_ref, bre_hbm, bim_hbm,
            cre_hbm, cim_hbm, ldt_ref, dsk_ref,
            o_hbm,
            x_s, w_s, wo_s, xb_s, bre_s, bim_s, cre_s, cim_s, o_s, sems,
            wt_s, qt_s, vt_s, kp_s, sA, sB, mA, mB, ot_s, ls_s, u_s, cp_s, kf_s, qf_s, par_s):
    j = pl.program_id(0)

    def rows_copy(src, dst, i, sem0):
        rows = pl.ds(pl.multiple_of(i * TQ, TQ), TQ)
        return pltpu.make_async_copy(src.at[rows], dst.at[rows], sems.at[sem0 + i])

    x_copy = lambda i: rows_copy(x_hbm, x_s, i, S_X0)
    xb_copy = lambda i: rows_copy(xb_hbm, xb_s, i, S_XB0)

    whole = {
        S_WQ: (wqkv_hbm.at[:, 0:DM], w_s.at[0]), S_WK: (wqkv_hbm.at[:, DM:2 * DM], w_s.at[1]),
        S_WV: (wqkv_hbm.at[:, 2 * DM:3 * DM], w_s.at[2]),
        S_BRE: (bre_hbm, bre_s), S_BIM: (bim_hbm, bim_s),
        S_CRE: (cre_hbm, cre_s), S_CIM: (cim_hbm, cim_s), S_WO: (wo_hbm, wo_s),
    }

    def copy(k):
        src, dst = whole[k]
        return pltpu.make_async_copy(src, dst, sems.at[k])

    def out_copy(step, half):
        slot = step % 2
        rows = pl.ds(pl.multiple_of(step * TQ, TQ), TQ)
        cols = pl.ds(half * DM, DM)
        return pltpu.make_async_copy(o_s.at[slot, :, cols], o_hbm.at[rows, cols],
                                     sems.at[S_OUT + 2 * slot + half])

    def head_rows(head):
        return pl.ds(pl.multiple_of(head * DH, DH), DH)

    def get_w(g, t):
        q = qt_s[g // PPB, head_rows((g % PPB) * UN + t), :]

        def pad(q):
            parts = [jnp.zeros((DH, TQ), BF16)] * KG
            parts[t % KG] = q
            return jnp.concatenate(parts, axis=0)

        w0 = pad(q)

        def make(z):
            if z is None:
                return w0
            zz = jnp.concatenate([z] * (TQ // 128), axis=1)[None]
            qz = q.astype(F32).reshape(DH // 8, 8, TQ) + zz
            return pad(qz.reshape(DH, TQ).astype(BF16))
        return make

    def qk_chunk(g, t, w, c, s_ref, macc, nrows):
        grp = (g % PPB) * (UN // KG) + t // KG
        s = _dot(kp_s[grp, c * CK:c * CK + nrows, :], w)
        s_ref[t, c * CK:c * CK + nrows, :] = s
        if nrows == CK:
            r = _red(s, jnp.max)
        else:
            r = jnp.max(s.reshape(nrows // VR, VR, TQ), axis=0)
        return r if macc is None else jnp.maximum(macc, r)

    def qk_vpu(g, t, c, s_ref, zin):
        kf = kf_s[g % PPB, c * VR:(c + 1) * VR, :]
        if zin is not None:
            kf = (kf.reshape(VR // 8, 8, 128) + zin[None]).reshape(VR, 128)
        s = None
        for d in range(DH):
            col = t * DH + d
            qb = jnp.concatenate(
                [jnp.broadcast_to(qf_s[g, col:col + 1, qt * 128:(qt + 1) * 128], (8, 128))
                 for qt in range(TQ // 128)], axis=1)
            kb = jnp.broadcast_to(kf[:, col:col + 1], (VR, TQ)).reshape(VR // 8, 8, TQ)
            p = kb * qb[None]
            s = p if s is None else s + p
        s = s.reshape(VR, TQ)
        s_ref[t, (c + 1) * CK - VR:(c + 1) * CK, :] = s
        return s

    def ex_chunk(m, t, c, s_ref, lacc):
        s = s_ref[t, c * CK:(c + 1) * CK, :].reshape(CK // 8, 8, TQ)
        p = jnp.exp2(s - m[None]).reshape(CK, TQ)
        r = _red(p, jnp.sum)
        return p.astype(BF16), (r if lacc is None else lacc + r)

    def pv_chunk(g, t, c, p, oacc, z):
        k0 = c * CK
        vt = vt_s[k0 // TQ, head_rows((g % PPB) * UN + t), k0 % TQ:k0 % TQ + CK]
        if z is not None:
            vt = (vt.astype(F32).reshape(DH // 8, 8, CK) + z[None]).reshape(DH, CK).astype(BF16)
        o = _dot(vt, p)
        return o if oacc is None else oacc + o

    def phase(ph, N_, C_, do_qk=True, do_pv=True, pre_qk=None, side=None):
        sN, mN = N_
        sC, mC = C_
        steps = [(t, c) for t in range(UN) for c in range(NC)]
        n = len(steps)
        ws, ms, laccs, ps = {}, {}, {}, {}
        macc = oacc = None
        hist = []
        pv_dep = {}

        def do_exp(i):
            t, c = steps[i]
            if c == 0:
                ms[t] = jnp.broadcast_to(mC[t], (8, TQ))
                laccs[t] = None
            ps[i], laccs[t] = ex_chunk(ms[t], t, c, sC, laccs[t])

        if do_pv:
            for i in range(min(LEAD, n)):
                do_exp(i)
        for i, (t, c) in enumerate(steps):
            if do_qk:
                if c == 0:
                    ws[t] = get_w(ph + 1, t)
                    macc = None
                z = pre_qk(i, hist) if pre_qk is not None else None
                off = do_pv and (c in OFFC)
                macc = qk_chunk(ph + 1, t, ws[t](z), c, sN, macc, CK - VR if off else CK)
                hist.append(macc[0:8, 0:128])
                if off:
                    zin = _zero_of(hist[i - LA]) if i >= LA else None
                    sv = qk_vpu(ph + 1, t, c, sN, zin)
                    macc = jnp.maximum(macc, sv)
                    pv_dep[i + LB] = _zero_of(sv[0:8, 0:128] + sv[8:16, 128:256])
                if c == NC - 1:
                    mN[t] = jnp.max(macc, axis=0, keepdims=True)
            if side is not None:
                side(i)
            if do_pv:
                if i + LEAD < n:
                    do_exp(i + LEAD)
                if c == 0:
                    oacc = None
                oacc = pv_chunk(ph, t, c, ps.pop(i), oacc, pv_dep.get(i))
                if c == NC - 1:
                    head = (ph % PPB) * UN + t
                    ot_s[head] = oacc
                    ls_s[head] = jnp.sum(laccs[t], axis=0, keepdims=True)

    A = (sA, mA)
    B = (sB, mB)

    def ssm_params():
        row1 = lambda ref: ref[...].astype(F32).reshape(1, DM)
        lam_re = row1(lre_ref)
        lam_im = row1(lim_ref)
        dt = jnp.exp(row1(ldt_ref)).astype(BF16).astype(F32)
        mag = jnp.exp(dt * lam_re)
        ang = dt * lam_im
        lb_re = mag * jnp.cos(ang)
        lb_im = mag * jnp.sin(ang)
        den = lam_re * lam_re + lam_im * lam_im
        nre = lb_re - 1.0
        par_s[0] = lb_re
        par_s[1] = lb_im
        par_s[2] = (nre * lam_re + lb_im * lam_im) / den
        par_s[3] = (lb_im * lam_re - nre * lam_im) / den

    def c_rows(r0, r1):
        co_re, co_im = par_s[2], par_s[3]
        cre = cre_s[r0:r1, :].astype(F32)
        cim = cim_s[r0:r1, :].astype(F32)
        a = 2.0 * (cre * co_re - cim * co_im)
        b = -2.0 * (cre * co_im + cim * co_re)
        cp_s[r0:r1, 0:DM] = a.astype(BF16)
        cp_s[r0:r1, DM:2 * DM] = b.astype(BF16)
        return a[0:8, 0:128]

    def scan_step(s, st, ar, ai, store):
        st = list(st)
        for lt in range(NLT):
            hr, hi = st[lt], st[NLT + lt]
            ur = u_s[lt, pl.ds(s, NCHUNK, stride=CLEN), :]
            ui = u_s[NLT + lt, pl.ds(s, NCHUNK, stride=CLEN), :]
            nr = ar[lt] * hr - ai[lt] * hi + ur
            ni = ar[lt] * hi + ai[lt] * hr + ui
            if store:
                u_s[lt, pl.ds(s, NCHUNK, stride=CLEN), :] = nr
                u_s[NLT + lt, pl.ds(s, NCHUNK, stride=CLEN), :] = ni
            st[lt], st[NLT + lt] = nr, ni
        return tuple(st)

    def chunk_carry(ends, ar, ai):
        row = jax.lax.broadcasted_iota(jnp.int32, (NCHUNK, 128), 0)
        init = []
        for lt in range(NLT):
            br, bi = ar[lt], ai[lt]
            pr = pi = None
            e = CLEN
            while e:
                if e & 1:
                    pr, pi = (br, bi) if pr is None else _cmul(pr, pi, br, bi)
                e >>= 1
                if e:
                    br, bi = _cmul(br, bi, br, bi)
            hr = jnp.where(row >= 1, pltpu.roll(ends[lt], 1, 0), 0.0)
            hi = jnp.where(row >= 1, pltpu.roll(ends[NLT + lt], 1, 0), 0.0)
            sh = 1
            while sh < NCHUNK:
                sr = jnp.where(row >= sh, pltpu.roll(hr, sh, 0), 0.0)
                si = jnp.where(row >= sh, pltpu.roll(hi, sh, 0), 0.0)
                dr, di = _cmul(pr, pi, sr, si)
                hr, hi = hr + dr, hi + di
                pr, pi = _cmul(pr, pi, pr, pi)
                sh *= 2
            init.append((hr, hi))
        return tuple(h[0] for h in init) + tuple(h[1] for h in init)

    class PacedScan:
        def __init__(self, nslices):
            lb_re, lb_im = par_s[0], par_s[1]
            tile = lambda v, lt: jnp.broadcast_to(v[:, lt * 128:(lt + 1) * 128], (NCHUNK, 128))
            self.ar = [tile(lb_re, lt) for lt in range(NLT)]
            self.ai = [tile(lb_im, lt) for lt in range(NLT)]
            self.st = tuple(jnp.zeros((NCHUNK, 128), F32) for _ in range(2 * NLT))
            self.items = [(False, s) for s in range(CLEN)] + [None] + [(True, s) for s in range(CLEN)]
            self.n = nslices
            self.crows = {(k * nslices) // (DM // 32): k for k in range(DM // 32)}

        def __call__(self, i, hist):
            lo = (i * len(self.items)) // self.n
            hi = ((i + 1) * len(self.items)) // self.n
            if i >= LAG:
                zin = _zero_of(hist[i - LAG])
                self.st = tuple(h + zin for h in self.st[:NLT]) + tuple(self.st[NLT:])
            for it in self.items[lo:hi]:
                if it is None:
                    self.st = chunk_carry(self.st, self.ar, self.ai)
                else:
                    self.st = scan_step(it[1], self.st, self.ar, self.ai, it[0])
            dep = (self.st[0] + self.st[1]) + (self.st[2] + self.st[3])
            if i in self.crows:
                k = self.crows[i]
                dep = dep + c_rows(32 * k, 32 * (k + 1))
            return _zero_of(dep)

    def proj_ssm_half(i, b_s, lt0):
        r0 = pl.multiple_of(i * TQ, TQ)
        u = _dot(xb_s[pl.ds(r0, TQ), :], b_s[...], _NT)
        for lt in range(NLT):
            u_s[lt0 + lt, pl.ds(r0, TQ), :] = u[:, lt * 128:(lt + 1) * 128]

    def proj_ssm_block(i):
        proj_ssm_half(i, bre_s, 0)
        proj_ssm_half(i, bim_s, NLT)

    def proj_attn_block(i):
        r0 = pl.multiple_of(i * TQ, TQ)
        xc = x_s[pl.ds(r0, TQ), :]
        q = _dot(wt_s[0], xc, _NT).astype(BF16)
        qt = (q.astype(F32) * QSCALE).astype(BF16)
        qt_s[i] = qt
        for hq in range(PPB):
            qf_s[i * PPB + hq] = qt[hq * UN * DH:(hq + 1) * UN * DH, :].astype(F32)
        vt_s[i] = _dot(wt_s[1], xc, _NT).astype(BF16)
        k = _dot(xc, w_s[1]).astype(BF16)
        for p in range(NHEAD // KG):
            kp_s[p, pl.ds(r0, TQ), :] = k[:, DH * KG * p:DH * KG * (p + 1)]
        for cc in range(TQ // CK):
            kr = k[(cc + 1) * CK - VR:(cc + 1) * CK, :].astype(F32)
            row = pl.multiple_of((i * (TQ // CK) + cc) * VR, VR)
            for lt in range(NLT):
                kf_s[lt, pl.ds(row, VR), :] = kr[:, lt * 128:(lt + 1) * 128]

    NPAIR = NQB // PU

    @pl.when(j == 0)
    def _prologue():
        copy(S_BRE).start()
        xb_copy(0).start()
        ssm_params()
        copy(S_BIM).start()
        xb_copy(1).start()
        for lt in range(2 * NLT):
            u_s[lt, SEQ:UROWS, :] = jnp.zeros((UROWS - SEQ, 128), F32)
        copy(S_BRE).wait()
        xb_copy(0).wait()
        proj_ssm_half(0, bre_s, 0)
        copy(S_BIM).wait()
        for r in range(PU, NQB):
            xb_copy(r).start()
        proj_ssm_half(0, bim_s, NLT)
        xb_copy(1).wait()
        proj_ssm_block(1)

        def proj_ssm(i, carry):
            for u in range(PU):
                xb_copy(i * PU + u).wait()

            @pl.when(i == 1)
            def _():
                for k in (S_WQ, S_WV, S_WK):
                    copy(k).start()
                for r in range(NQB):
                    x_copy(r).start()

            for u in range(PU):
                proj_ssm_block(i * PU + u)
            return carry
        jax.lax.fori_loop(1, NPAIR - 1, proj_ssm, 0)

        for u in range(PU):
            xb_copy(NQB - PU + u).wait()
        copy(S_WQ).wait()
        copy(S_WV).wait()
        for k in (S_CRE, S_CIM, S_WO):
            copy(k).start()
        for u in range(PU):
            proj_ssm_block(NQB - PU + u)
            wt_s[u] = w_s[2 * u].T
        copy(S_WK).wait()

        def proj_attn(i, carry):
            for u in range(PU):
                x_copy(i * PU + u).wait()
            for u in range(PU):
                proj_attn_block(i * PU + u)
            return carry
        jax.lax.fori_loop(0, NPAIR, proj_attn, 0)

        for k in (S_CRE, S_CIM, S_WO):
            copy(k).wait()

    @pl.when(j == 0)
    def _fill():
        phase(-1, A, B, do_pv=False, pre_qk=PacedScan(UN * NC))

    def one_phase(i, carry):
        ph = j * PPB + i

        @pl.when(i % 2 == 0)
        def _even():
            phase(ph, B, A)

        @pl.when(i % 2 == 1)
        def _odd():
            phase(ph, A, B)
        return carry

    nph = jnp.where(j == NQB - 1, PPB - 1, PPB)
    jax.lax.fori_loop(0, nph, one_phase, 0)

    slot = j % 2

    @pl.when(j >= 2)
    def _free_slot():
        out_copy(j - 2, 0).wait()
        out_copy(j - 2, 1).wait()

    def ssm_out():
        r0 = pl.multiple_of(j * TQ, TQ)
        g = jnp.concatenate([u_s[lt, pl.ds(r0, TQ), :] for lt in range(2 * NLT)], axis=1).astype(BF16)
        y = _dot(g, cp_s[...], _NT)
        d = dsk_ref[...].astype(F32).reshape(1, DM)
        o_s[slot, :, DM:2 * DM] = y + xb_s[pl.ds(r0, TQ), :].astype(F32) * d

    def attn_out():
        o = (ot_s[...] * (1.0 / ls_s[...])).reshape(DM, TQ).astype(BF16)
        o_s[slot, :, 0:DM] = _dot(o, wo_s[...], _TN)

    class SsmOutPieces:
        def __init__(self, nsteps):
            self.r0 = (NQB - 1) * TQ
            self.npieces = NLT * 2 * NLT
            self.at = {(p * nsteps) // self.npieces: p for p in range(self.npieces)}
            self.acc = None

        def __call__(self, i):
            if i not in self.at:
                return
            n, k = divmod(self.at[i], 2 * NLT)
            g = u_s[k, self.r0:self.r0 + TQ, :].astype(BF16)
            part = _dot(g, cp_s[n * 128:(n + 1) * 128, k * 128:(k + 1) * 128], _NT)
            self.acc = part if k == 0 else self.acc + part
            if k == 2 * NLT - 1:
                d = dsk_ref[...].astype(F32).reshape(1, DM)[:, n * 128:(n + 1) * 128]
                xb = xb_s[self.r0:self.r0 + TQ, n * 128:(n + 1) * 128].astype(F32)
                o_s[(NQB - 1) % 2, :, DM + n * 128:DM + (n + 1) * 128] = self.acc + xb * d

    @pl.when(j < NQB - 1)
    def _notlast():
        ssm_out()
        attn_out()
        out_copy(j, 0).start()
        out_copy(j, 1).start()

    @pl.when(j == NQB - 1)
    def _last():
        phase(NPH - 1, A, B, do_qk=False, side=SsmOutPieces(UN * NC))
        out_copy(j, 1).start()

    @pl.when(j == NQB - 1)
    def _last2():
        attn_out()
        out_copy(j, 0).start()
        out_copy(j - 1, 0).wait()
        out_copy(j - 1, 1).wait()
        out_copy(j, 1).wait()
        out_copy(j, 0).wait()


@jax.jit
def pallas_concat_heads__softmax_full_mha__ssm_conv_s5__prompt_kernel(
    A_x, A_wqkv, A_wo, B_x, B_Lambda_re, B_Lambda_im, B_B_re, B_B_im, B_C_re, B_C_im,
    B_log_dt, B_Dskip,
):
    hbm = pl.BlockSpec(memory_space=pl.ANY)
    vec = pl.BlockSpec((DM,), lambda j: (0,))
    args = (A_x.reshape(SEQ, DM), A_wqkv, A_wo, B_x.reshape(SEQ, DM), B_Lambda_re,
            B_Lambda_im, B_B_re, B_B_im, B_C_re, B_C_im, B_log_dt, B_Dskip)
    in_specs = [hbm, hbm, hbm, hbm, vec, vec, hbm, hbm, hbm, hbm, vec, vec]
    scratch = [
        pltpu.VMEM((SEQ, DM), BF16),
        pltpu.VMEM((3, DM, DM), BF16),
        pltpu.VMEM((DM, DM), BF16),
        pltpu.VMEM((SEQ, DM), BF16),
        pltpu.VMEM((DM, DM), BF16),
        pltpu.VMEM((DM, DM), BF16),
        pltpu.VMEM((DM, DM), BF16),
        pltpu.VMEM((DM, DM), BF16),
        pltpu.VMEM((2, TQ, 2 * DM), F32),
        pltpu.SemaphoreType.DMA((NSEM,)),
        pltpu.VMEM((2, DM, DM), BF16),
        pltpu.VMEM((NQB, DM, TQ), BF16),
        pltpu.VMEM((NQB, DM, TQ), BF16),
        pltpu.VMEM((NHEAD // KG, SEQ, DH * KG), BF16),
        pltpu.VMEM((UN, SEQ, TQ), F32),
        pltpu.VMEM((UN, SEQ, TQ), F32),
        pltpu.VMEM((UN, 1, TQ), F32),
        pltpu.VMEM((UN, 1, TQ), F32),
        pltpu.VMEM((NHEAD, DH, TQ), F32),
        pltpu.VMEM((NHEAD, 1, TQ), F32),
        pltpu.VMEM((2 * NLT, UROWS, 128), F32),
        pltpu.VMEM((DM, 2 * DM), BF16),
        pltpu.VMEM((NLT, NC * VR, 128), F32),
        pltpu.VMEM((NPH, UN * DH, TQ), F32),
        pltpu.VMEM((4, 1, DM), F32),
    ]
    out = pl.pallas_call(
        _kernel,
        grid=(NQB,),
        in_specs=in_specs,
        out_specs=pl.BlockSpec(memory_space=pl.ANY),
        out_shape=jax.ShapeDtypeStruct((SEQ, 2 * DM), F32),
        scratch_shapes=scratch,
        compiler_params=pltpu.CompilerParams(
            dimension_semantics=("arbitrary",),
            vmem_limit_bytes=110 * 1024 * 1024),
    )(*args)
    return out.reshape(1, SEQ, 2 * DM)
```

```python
import math

import jax
import jax.numpy as jnp
import jax.experimental.pallas as pl
import jax.experimental.pallas.tpu as pltpu

F32 = jnp.float32
BF16 = jnp.bfloat16

SEQ = 2048
DM = 512
NHEAD = 32
DH = 16
TQ = 256
NQB = SEQ // TQ
UN = 8
PPB = NHEAD // UN
NPH = NQB * PPB
CK = 128
NC = SEQ // CK
NACC = 2
KG = 4
LEAD = 2
VR = 16
OFFC = (1, 3, 6, 8, 11, 13)
LA = 3
LB = 9
LAG = 8
PU = 2
PA = 4
NCHUNK = 8
CLEN = SEQ // NCHUNK + 1
UROWS = NCHUNK * CLEN
NLT = DM // 128
QSCALE = (DH ** -0.5) * math.log2(math.e)

_NN = (((1,), (0,)), ((), ()))
_NT = (((1,), (1,)), ((), ()))
_TN = (((0,), (0,)), ((), ()))

S_WQ, S_WK, S_WV, S_BRE, S_BIM, S_CRE, S_CIM, S_WO, S_X0 = range(9)
S_XB0 = S_X0 + NQB
S_OUT = S_XB0 + NQB
NSEM = S_OUT + 4


def _dot(a, b, dims=_NN):
    return jax.lax.dot_general(a, b, dims, preferred_element_type=F32)


def _red(x, op):
    r = x.shape[0]
    return op(x.reshape(r // (8 * NACC), 8 * NACC, x.shape[1]), axis=0)


def _zero_of(v):
    i = v.astype(jnp.int32)
    i = jax.lax.shift_right_logical(jax.lax.shift_right_logical(i, 31), 1)
    return i.astype(F32)


def _cmul(ar, ai, br, bi):
    return ar * br - ai * bi, ar * bi + ai * br


def _kernel(x_hbm, wqkv_hbm, wo_hbm, xb_hbm, lre_ref, lim_ref, bre_hbm, bim_hbm,
            cre_hbm, cim_hbm, ldt_ref, dsk_ref,
            o_hbm,
            x_s, w_s, wo_s, xb_s, bre_s, bim_s, cre_s, cim_s, o_s, sems,
            wt_s, qt_s, vt_s, kp_s, sA, sB, mA, mB, ot_s, ls_s, u_s, cp_s, kf_s, qf_s, par_s):
    j = pl.program_id(0)

    def rows_copy(src, dst, i, sem0):
        rows = pl.ds(pl.multiple_of(i * TQ, TQ), TQ)
        return pltpu.make_async_copy(src.at[rows], dst.at[rows], sems.at[sem0 + i])

    x_copy = lambda i: rows_copy(x_hbm, x_s, i, S_X0)
    xb_copy = lambda i: rows_copy(xb_hbm, xb_s, i, S_XB0)

    whole = {
        S_WQ: (wqkv_hbm.at[:, 0:DM], w_s.at[0]), S_WK: (wqkv_hbm.at[:, DM:2 * DM], w_s.at[1]),
        S_WV: (wqkv_hbm.at[:, 2 * DM:3 * DM], w_s.at[2]),
        S_BRE: (bre_hbm, bre_s), S_BIM: (bim_hbm, bim_s),
        S_CRE: (cre_hbm, cre_s), S_CIM: (cim_hbm, cim_s), S_WO: (wo_hbm, wo_s),
    }

    def copy(k):
        src, dst = whole[k]
        return pltpu.make_async_copy(src, dst, sems.at[k])

    def out_copy(step, half):
        slot = step % 2
        rows = pl.ds(pl.multiple_of(step * TQ, TQ), TQ)
        cols = pl.ds(half * DM, DM)
        return pltpu.make_async_copy(o_s.at[slot, :, cols], o_hbm.at[rows, cols],
                                     sems.at[S_OUT + 2 * slot + half])

    def head_rows(head):
        return pl.ds(pl.multiple_of(head * DH, DH), DH)

    def get_w(grp, t):
        _, qb, hq = grp
        q = qt_s[qb, head_rows(hq * UN + t), :]

        def pad(q):
            parts = [jnp.zeros((DH, TQ), BF16)] * KG
            parts[t % KG] = q
            return jnp.concatenate(parts, axis=0)

        w0 = pad(q)

        def make(z):
            if z is None:
                return w0
            zz = jnp.concatenate([z] * (TQ // 128), axis=1)[None]
            qz = q.astype(F32).reshape(DH // 8, 8, TQ) + zz
            return pad(qz.reshape(DH, TQ).astype(BF16))
        return make

    def qk_chunk(grp, t, w, c, s_ref, macc, nrows):
        karr = grp[2] * (UN // KG) + t // KG
        s = _dot(kp_s[karr, c * CK:c * CK + nrows, :], w)
        s_ref[t, c * CK:c * CK + nrows, :] = s
        if nrows == CK:
            r = _red(s, jnp.max)
        else:
            r = jnp.max(s.reshape(nrows // VR, VR, TQ), axis=0)
        return r if macc is None else jnp.maximum(macc, r)

    def qk_vpu(grp, t, c, s_ref, zin):
        g, _, hq = grp
        kf = kf_s[hq, c * VR:(c + 1) * VR, :]
        if zin is not None:
            kf = (kf.reshape(VR // 8, 8, 128) + zin[None]).reshape(VR, 128)
        s = None
        for d in range(DH):
            col = t * DH + d
            qb = jnp.concatenate(
                [jnp.broadcast_to(qf_s[g, col:col + 1, qt * 128:(qt + 1) * 128], (8, 128))
                 for qt in range(TQ // 128)], axis=1)
            kb = jnp.broadcast_to(kf[:, col:col + 1], (VR, TQ)).reshape(VR // 8, 8, TQ)
            p = kb * qb[None]
            s = p if s is None else s + p
        s = s.reshape(VR, TQ)
        s_ref[t, (c + 1) * CK - VR:(c + 1) * CK, :] = s
        return s

    def ex_chunk(m, t, c, s_ref, lacc):
        s = s_ref[t, c * CK:(c + 1) * CK, :].reshape(CK // 8, 8, TQ)
        p = jnp.exp2(s - m[None]).reshape(CK, TQ)
        r = _red(p, jnp.sum)
        return p.astype(BF16), (r if lacc is None else lacc + r)

    def pv_chunk(grp, t, c, p, oacc, z):
        k0 = c * CK
        vt = vt_s[k0 // TQ, head_rows(grp[2] * UN + t), k0 % TQ:k0 % TQ + CK]
        if z is not None:
            vt = (vt.astype(F32).reshape(DH // 8, 8, CK) + z[None]).reshape(DH, CK).astype(BF16)
        o = _dot(vt, p)
        return o if oacc is None else oacc + o

    def phase(ph, N_, C_, do_qk=True, do_pv=True, pre_qk=None, side=None):
        sN, mN = N_
        sC, mC = C_
        steps = [(t, c) for t in range(UN) for c in range(NC)]
        n = len(steps)
        ws, ms, laccs, ps = {}, {}, {}, {}
        macc = oacc = None
        hist = []
        pv_dep = {}
        cur = (ph, ph // PPB, ph % PPB)
        nxt = (ph + 1, (ph + 1) // PPB, (ph + 1) % PPB)

        def do_exp(i):
            t, c = steps[i]
            if c == 0:
                ms[t] = jnp.broadcast_to(mC[t], (8, TQ))
                laccs[t] = None
            ps[i], laccs[t] = ex_chunk(ms[t], t, c, sC, laccs[t])

        if do_pv:
            for i in range(min(LEAD, n)):
                do_exp(i)
        for i, (t, c) in enumerate(steps):
            if do_qk:
                if c == 0:
                    ws[t] = get_w(nxt, t)
                    macc = None
                z = pre_qk(i, hist) if pre_qk is not None else None
                off = do_pv and (c in OFFC)
                macc = qk_chunk(nxt, t, ws[t](z), c, sN, macc, CK - VR if off else CK)
                hist.append(macc[0:8, 0:128])
                if off:
                    zin = _zero_of(hist[i - LA]) if i >= LA else None
                    sv = qk_vpu(nxt, t, c, sN, zin)
                    macc = jnp.maximum(macc, sv)
                    pv_dep[i + LB] = _zero_of(sv[0:8, 0:128] + sv[8:16, 128:256])
                if c == NC - 1:
                    mN[t] = jnp.max(macc, axis=0, keepdims=True)
            if side is not None:
                side(i)
            if do_pv:
                if i + LEAD < n:
                    do_exp(i + LEAD)
                if c == 0:
                    oacc = None
                oacc = pv_chunk(cur, t, c, ps.pop(i), oacc, pv_dep.get(i))
                if c == NC - 1:
                    head = cur[2] * UN + t
                    ot_s[head] = oacc
                    ls_s[head] = jnp.sum(laccs[t], axis=0, keepdims=True)

    A = (sA, mA)
    B = (sB, mB)

    def ssm_params():
        row1 = lambda ref: ref[...].astype(F32).reshape(1, DM)
        lam_re = row1(lre_ref)
        lam_im = row1(lim_ref)
        dt = jnp.exp(row1(ldt_ref)).astype(BF16).astype(F32)
        mag = jnp.exp(dt * lam_re)
        ang = dt * lam_im
        lb_re = mag * jnp.cos(ang)
        lb_im = mag * jnp.sin(ang)
        den = lam_re * lam_re + lam_im * lam_im
        nre = lb_re - 1.0
        par_s[0] = lb_re
        par_s[1] = lb_im
        par_s[2] = (nre * lam_re + lb_im * lam_im) / den
        par_s[3] = (lb_im * lam_re - nre * lam_im) / den

    def c_rows(r0, r1):
        co_re, co_im = par_s[2], par_s[3]
        cre = cre_s[r0:r1, :].astype(F32)
        cim = cim_s[r0:r1, :].astype(F32)
        a = 2.0 * (cre * co_re - cim * co_im)
        b = -2.0 * (cre * co_im + cim * co_re)
        cp_s[r0:r1, 0:DM] = a.astype(BF16)
        cp_s[r0:r1, DM:2 * DM] = b.astype(BF16)
        return a[0:8, 0:128]

    def scan_step(s, st, ar, ai, store):
        st = list(st)
        for lt in range(NLT):
            hr, hi = st[lt], st[NLT + lt]
            ur = u_s[lt, pl.ds(s, NCHUNK, stride=CLEN), :]
            ui = u_s[NLT + lt, pl.ds(s, NCHUNK, stride=CLEN), :]
            nr = ar[lt] * hr - ai[lt] * hi + ur
            ni = ar[lt] * hi + ai[lt] * hr + ui
            if store:
                u_s[lt, pl.ds(s, NCHUNK, stride=CLEN), :] = nr
                u_s[NLT + lt, pl.ds(s, NCHUNK, stride=CLEN), :] = ni
            st[lt], st[NLT + lt] = nr, ni
        return tuple(st)

    def chunk_carry(ends, ar, ai):
        row = jax.lax.broadcasted_iota(jnp.int32, (NCHUNK, 128), 0)
        init = []
        for lt in range(NLT):
            br, bi = ar[lt], ai[lt]
            pr = pi = None
            e = CLEN
            while e:
                if e & 1:
                    pr, pi = (br, bi) if pr is None else _cmul(pr, pi, br, bi)
                e >>= 1
                if e:
                    br, bi = _cmul(br, bi, br, bi)
            hr = jnp.where(row >= 1, pltpu.roll(ends[lt], 1, 0), 0.0)
            hi = jnp.where(row >= 1, pltpu.roll(ends[NLT + lt], 1, 0), 0.0)
            sh = 1
            while sh < NCHUNK:
                sr = jnp.where(row >= sh, pltpu.roll(hr, sh, 0), 0.0)
                si = jnp.where(row >= sh, pltpu.roll(hi, sh, 0), 0.0)
                dr, di = _cmul(pr, pi, sr, si)
                hr, hi = hr + dr, hi + di
                pr, pi = _cmul(pr, pi, pr, pi)
                sh *= 2
            init.append((hr, hi))
        return tuple(h[0] for h in init) + tuple(h[1] for h in init)

    class PacedScan:
        def __init__(self, nslices):
            lb_re, lb_im = par_s[0], par_s[1]
            tile = lambda v, lt: jnp.broadcast_to(v[:, lt * 128:(lt + 1) * 128], (NCHUNK, 128))
            self.ar = [tile(lb_re, lt) for lt in range(NLT)]
            self.ai = [tile(lb_im, lt) for lt in range(NLT)]
            self.st = tuple(jnp.zeros((NCHUNK, 128), F32) for _ in range(2 * NLT))
            self.items = [(False, s) for s in range(CLEN)] + [None] + [(True, s) for s in range(CLEN)]
            self.n = nslices
            self.crows = {(k * nslices) // (DM // 32): k for k in range(DM // 32)}

        def __call__(self, i, hist):
            lo = (i * len(self.items)) // self.n
            hi = ((i + 1) * len(self.items)) // self.n
            if i >= LAG:
                zin = _zero_of(hist[i - LAG])
                self.st = tuple(h + zin for h in self.st[:NLT]) + tuple(self.st[NLT:])
            for it in self.items[lo:hi]:
                if it is None:
                    self.st = chunk_carry(self.st, self.ar, self.ai)
                else:
                    self.st = scan_step(it[1], self.st, self.ar, self.ai, it[0])
            dep = (self.st[0] + self.st[1]) + (self.st[2] + self.st[3])
            if i in self.crows:
                k = self.crows[i]
                dep = dep + c_rows(32 * k, 32 * (k + 1))
            return _zero_of(dep)

    def proj_ssm_half(i, b_s, lt0):
        r0 = pl.multiple_of(i * TQ, TQ)
        u = _dot(xb_s[pl.ds(r0, TQ), :], b_s[...], _NT)
        for lt in range(NLT):
            u_s[lt0 + lt, pl.ds(r0, TQ), :] = u[:, lt * 128:(lt + 1) * 128]

    def proj_ssm_block(i):
        proj_ssm_half(i, bre_s, 0)
        proj_ssm_half(i, bim_s, NLT)

    def proj_attn_block(i):
        r0 = pl.multiple_of(i * TQ, TQ)
        xc = x_s[pl.ds(r0, TQ), :]
        q = _dot(wt_s[0], xc, _NT).astype(BF16)
        qt = (q.astype(F32) * QSCALE).astype(BF16)
        qt_s[i] = qt
        for hq in range(PPB):
            qf_s[i * PPB + hq] = qt[hq * UN * DH:(hq + 1) * UN * DH, :].astype(F32)
        vt_s[i] = _dot(wt_s[1], xc, _NT).astype(BF16)
        k = _dot(xc, w_s[1]).astype(BF16)
        for p in range(NHEAD // KG):
            kp_s[p, pl.ds(r0, TQ), :] = k[:, DH * KG * p:DH * KG * (p + 1)]
        for cc in range(TQ // CK):
            kr = k[(cc + 1) * CK - VR:(cc + 1) * CK, :].astype(F32)
            row = pl.multiple_of((i * (TQ // CK) + cc) * VR, VR)
            for lt in range(NLT):
                kf_s[lt, pl.ds(row, VR), :] = kr[:, lt * 128:(lt + 1) * 128]

    NPAIR = NQB // PU

    @pl.when(j == 0)
    def _prologue():
        copy(S_BRE).start()
        xb_copy(0).start()
        ssm_params()
        copy(S_BIM).start()
        xb_copy(1).start()
        for lt in range(2 * NLT):
            u_s[lt, SEQ:UROWS, :] = jnp.zeros((UROWS - SEQ, 128), F32)
        copy(S_BRE).wait()
        xb_copy(0).wait()
        proj_ssm_half(0, bre_s, 0)
        copy(S_BIM).wait()
        for r in range(PU, NQB):
            xb_copy(r).start()
        proj_ssm_half(0, bim_s, NLT)
        xb_copy(1).wait()
        proj_ssm_block(1)

        def proj_ssm(i, carry):
            for u in range(PU):
                xb_copy(i * PU + u).wait()

            @pl.when(i == 1)
            def _():
                for k in (S_WQ, S_WV, S_WK):
                    copy(k).start()
                for r in range(NQB):
                    x_copy(r).start()

            for u in range(PU):
                proj_ssm_block(i * PU + u)
            return carry
        jax.lax.fori_loop(1, NPAIR - 1, proj_ssm, 0)

        for u in range(PU):
            xb_copy(NQB - PU + u).wait()
        copy(S_WQ).wait()
        copy(S_WV).wait()
        for k in (S_CRE, S_CIM, S_WO):
            copy(k).start()
        for u in range(PU):
            proj_ssm_block(NQB - PU + u)
            wt_s[u] = w_s[2 * u].T
        copy(S_WK).wait()

        def proj_attn(i, carry):
            for u in range(PA):
                x_copy(i * PA + u).wait()
            for u in range(PA):
                proj_attn_block(i * PA + u)
            return carry
        jax.lax.fori_loop(0, NQB // PA, proj_attn, 0)

        for k in (S_CRE, S_CIM, S_WO):
            copy(k).wait()

    @pl.when(j == 0)
    def _fill():
        phase(-1, A, B, do_pv=False, pre_qk=PacedScan(UN * NC))

    def one_phase(i, carry):
        ph = j * PPB + i

        @pl.when(i % 2 == 0)
        def _even():
            phase(ph, B, A)

        @pl.when(i % 2 == 1)
        def _odd():
            phase(ph, A, B)
        return carry

    nph = jnp.where(j == NQB - 1, PPB - 1, PPB)
    jax.lax.fori_loop(0, nph, one_phase, 0)

    slot = j % 2

    @pl.when(j >= 2)
    def _free_slot():
        out_copy(j - 2, 0).wait()
        out_copy(j - 2, 1).wait()

    def ssm_out():
        r0 = pl.multiple_of(j * TQ, TQ)
        g = jnp.concatenate([u_s[lt, pl.ds(r0, TQ), :] for lt in range(2 * NLT)], axis=1).astype(BF16)
        y = _dot(g, cp_s[...], _NT)
        d = dsk_ref[...].astype(F32).reshape(1, DM)
        o_s[slot, :, DM:2 * DM] = y + xb_s[pl.ds(r0, TQ), :].astype(F32) * d

    def attn_out():
        o = (ot_s[...] * (1.0 / ls_s[...])).reshape(DM, TQ).astype(BF16)
        o_s[slot, :, 0:DM] = _dot(o, wo_s[...], _TN)

    class SsmOutPieces:
        def __init__(self, nsteps):
            self.r0 = (NQB - 1) * TQ
            self.npieces = NLT * 2 * NLT
            self.at = {(p * nsteps) // self.npieces: p for p in range(self.npieces)}
            self.acc = None

        def __call__(self, i):
            if i not in self.at:
                return
            n, k = divmod(self.at[i], 2 * NLT)
            g = u_s[k, self.r0:self.r0 + TQ, :].astype(BF16)
            part = _dot(g, cp_s[n * 128:(n + 1) * 128, k * 128:(k + 1) * 128], _NT)
            self.acc = part if k == 0 else self.acc + part
            if k == 2 * NLT - 1:
                d = dsk_ref[...].astype(F32).reshape(1, DM)[:, n * 128:(n + 1) * 128]
                xb = xb_s[self.r0:self.r0 + TQ, n * 128:(n + 1) * 128].astype(F32)
                o_s[(NQB - 1) % 2, :, DM + n * 128:DM + (n + 1) * 128] = self.acc + xb * d

    @pl.when(j < NQB - 1)
    def _notlast():
        ssm_out()
        attn_out()
        out_copy(j, 0).start()
        out_copy(j, 1).start()

    @pl.when(j == NQB - 1)
    def _last():
        phase(NPH - 1, A, B, do_qk=False, side=SsmOutPieces(UN * NC))
        out_copy(j, 1).start()

    @pl.when(j == NQB - 1)
    def _last2():
        attn_out()
        out_copy(j, 0).start()
        out_copy(j - 1, 0).wait()
        out_copy(j - 1, 1).wait()
        out_copy(j, 1).wait()
        out_copy(j, 0).wait()


@jax.jit
def pallas_concat_heads__softmax_full_mha__ssm_conv_s5__prompt_kernel(
    A_x, A_wqkv, A_wo, B_x, B_Lambda_re, B_Lambda_im, B_B_re, B_B_im, B_C_re, B_C_im,
    B_log_dt, B_Dskip,
):
    hbm = pl.BlockSpec(memory_space=pl.ANY)
    vec = pl.BlockSpec((DM,), lambda j: (0,))
    args = (A_x.reshape(SEQ, DM), A_wqkv, A_wo, B_x.reshape(SEQ, DM), B_Lambda_re,
            B_Lambda_im, B_B_re, B_B_im, B_C_re, B_C_im, B_log_dt, B_Dskip)
    in_specs = [hbm, hbm, hbm, hbm, vec, vec, hbm, hbm, hbm, hbm, vec, vec]
    scratch = [
        pltpu.VMEM((SEQ, DM), BF16),
        pltpu.VMEM((3, DM, DM), BF16),
        pltpu.VMEM((DM, DM), BF16),
        pltpu.VMEM((SEQ, DM), BF16),
        pltpu.VMEM((DM, DM), BF16),
        pltpu.VMEM((DM, DM), BF16),
        pltpu.VMEM((DM, DM), BF16),
        pltpu.VMEM((DM, DM), BF16),
        pltpu.VMEM((2, TQ, 2 * DM), F32),
        pltpu.SemaphoreType.DMA((NSEM,)),
        pltpu.VMEM((2, DM, DM), BF16),
        pltpu.VMEM((NQB, DM, TQ), BF16),
        pltpu.VMEM((NQB, DM, TQ), BF16),
        pltpu.VMEM((NHEAD // KG, SEQ, DH * KG), BF16),
        pltpu.VMEM((UN, SEQ, TQ), F32),
        pltpu.VMEM((UN, SEQ, TQ), F32),
        pltpu.VMEM((UN, 1, TQ), F32),
        pltpu.VMEM((UN, 1, TQ), F32),
        pltpu.VMEM((NHEAD, DH, TQ), F32),
        pltpu.VMEM((NHEAD, 1, TQ), F32),
        pltpu.VMEM((2 * NLT, UROWS, 128), F32),
        pltpu.VMEM((DM, 2 * DM), BF16),
        pltpu.VMEM((NLT, NC * VR, 128), F32),
        pltpu.VMEM((NPH, UN * DH, TQ), F32),
        pltpu.VMEM((4, 1, DM), F32),
    ]
    out = pl.pallas_call(
        _kernel,
        grid=(NQB,),
        in_specs=in_specs,
        out_specs=pl.BlockSpec(memory_space=pl.ANY),
        out_shape=jax.ShapeDtypeStruct((SEQ, 2 * DM), F32),
        scratch_shapes=scratch,
        compiler_params=pltpu.CompilerParams(
            dimension_semantics=("arbitrary",),
            vmem_limit_bytes=110 * 1024 * 1024),
    )(*args)
    return out.reshape(1, SEQ, 2 * DM)
```

```python
import math

import jax
import jax.numpy as jnp
import jax.experimental.pallas as pl
import jax.experimental.pallas.tpu as pltpu

F32 = jnp.float32
BF16 = jnp.bfloat16

SEQ = 2048
DM = 512
NHEAD = 32
DH = 16
TQ = 256
NQB = SEQ // TQ
UN = 8
PPB = NHEAD // UN
NPH = NQB * PPB
CK = 128
NC = SEQ // CK
NACC = 2
KG = 4
LEAD = 2
VR = 16
OFFC = (1, 3, 6, 8, 11, 13)
LA = 3
LB = 9
LAG = 8
PU = 2
PA = 4
NCHUNK = 8
CLEN = SEQ // NCHUNK + 1
UROWS = NCHUNK * CLEN
NLT = DM // 128
QSCALE = (DH ** -0.5) * math.log2(math.e)

_NN = (((1,), (0,)), ((), ()))
_NT = (((1,), (1,)), ((), ()))
_TN = (((0,), (0,)), ((), ()))

S_WQ, S_WK, S_WV, S_BRE, S_BIM, S_CRE, S_CIM, S_WO, S_X0 = range(9)
S_XB0 = S_X0 + NQB
S_OUT = S_XB0 + NQB
NSEM = S_OUT + 4


def _dot(a, b, dims=_NN):
    return jax.lax.dot_general(a, b, dims, preferred_element_type=F32)


def _red(x, op):
    r = x.shape[0]
    return op(x.reshape(r // (8 * NACC), 8 * NACC, x.shape[1]), axis=0)


def _zero_of(v):
    i = v.astype(jnp.int32)
    i = jax.lax.shift_right_logical(jax.lax.shift_right_logical(i, 31), 1)
    return i.astype(F32)


def _cmul(ar, ai, br, bi):
    return ar * br - ai * bi, ar * bi + ai * br


def _kernel(x_hbm, wqkv_hbm, wo_hbm, xb_hbm, lre_ref, lim_ref, bre_hbm, bim_hbm,
            cre_hbm, cim_hbm, ldt_ref, dsk_ref,
            o_hbm,
            x_s, w_s, wo_s, xb_s, bre_s, bim_s, cre_s, cim_s, o_s, sems,
            wt_s, qt_s, vt_s, kp_s, sA, sB, mA, mB, ot_s, ls_s, u_s, cp_s, kf_s, qf_s, par_s):
    j = pl.program_id(0)

    def rows_copy(src, dst, i, sem0):
        rows = pl.ds(pl.multiple_of(i * TQ, TQ), TQ)
        return pltpu.make_async_copy(src.at[rows], dst.at[rows], sems.at[sem0 + i])

    x_copy = lambda i: rows_copy(x_hbm, x_s, i, S_X0)
    xb_copy = lambda i: rows_copy(xb_hbm, xb_s, i, S_XB0)

    whole = {
        S_WQ: (wqkv_hbm.at[:, 0:DM], w_s.at[0]), S_WK: (wqkv_hbm.at[:, DM:2 * DM], w_s.at[1]),
        S_WV: (wqkv_hbm.at[:, 2 * DM:3 * DM], w_s.at[2]),
        S_BRE: (bre_hbm, bre_s), S_BIM: (bim_hbm, bim_s),
        S_CRE: (cre_hbm, cre_s), S_CIM: (cim_hbm, cim_s), S_WO: (wo_hbm, wo_s),
    }

    def copy(k):
        src, dst = whole[k]
        return pltpu.make_async_copy(src, dst, sems.at[k])

    def out_copy(step, half):
        slot = step % 2
        rows = pl.ds(pl.multiple_of(step * TQ, TQ), TQ)
        cols = pl.ds(half * DM, DM)
        return pltpu.make_async_copy(o_s.at[slot, :, cols], o_hbm.at[rows, cols],
                                     sems.at[S_OUT + 2 * slot + half])

    def head_rows(head):
        return pl.ds(pl.multiple_of(head * DH, DH), DH)

    def get_w(grp, t):
        _, qb, hq = grp
        q = qt_s[qb, head_rows(hq * UN + t), :]

        def pad(q):
            parts = [jnp.zeros((DH, TQ), BF16)] * KG
            parts[t % KG] = q
            return jnp.concatenate(parts, axis=0)

        w0 = pad(q)

        def make(z):
            if z is None:
                return w0
            zz = jnp.concatenate([z] * (TQ // 128), axis=1)[None]
            qz = q.astype(F32).reshape(DH // 8, 8, TQ) + zz
            return pad(qz.reshape(DH, TQ).astype(BF16))
        return make

    def qk_chunk(grp, t, w, c, s_ref, macc, nrows):
        karr = grp[2] * (UN // KG) + t // KG
        s = _dot(kp_s[karr, c * CK:c * CK + nrows, :], w)
        s_ref[t, c * CK:c * CK + nrows, :] = s
        if nrows == CK:
            r = _red(s, jnp.max)
        else:
            r = jnp.max(s.reshape(nrows // VR, VR, TQ), axis=0)
        return r if macc is None else jnp.maximum(macc, r)

    def qk_vpu(grp, t, c, s_ref, zin):
        g, _, hq = grp
        kf = kf_s[hq, c * VR:(c + 1) * VR, :]
        if zin is not None:
            kf = (kf.reshape(VR // 8, 8, 128) + zin[None]).reshape(VR, 128)
        s = None
        for d in range(DH):
            col = t * DH + d
            qb = jnp.concatenate(
                [jnp.broadcast_to(qf_s[g, col:col + 1, qt * 128:(qt + 1) * 128], (8, 128))
                 for qt in range(TQ // 128)], axis=1)
            kb = jnp.broadcast_to(kf[:, col:col + 1], (VR, TQ)).reshape(VR // 8, 8, TQ)
            p = kb * qb[None]
            s = p if s is None else s + p
        s = s.reshape(VR, TQ)
        s_ref[t, (c + 1) * CK - VR:(c + 1) * CK, :] = s
        return s

    def ex_chunk(m, t, c, s_ref, lacc):
        s = s_ref[t, c * CK:(c + 1) * CK, :].reshape(CK // 8, 8, TQ)
        p = jnp.exp2(s - m[None]).reshape(CK, TQ)
        r = _red(p, jnp.sum)
        return p.astype(BF16), (r if lacc is None else lacc + r)

    def pv_chunk(grp, t, c, p, oacc, z):
        k0 = c * CK
        vt = vt_s[k0 // TQ, head_rows(grp[2] * UN + t), k0 % TQ:k0 % TQ + CK]
        if z is not None:
            vt = (vt.astype(F32).reshape(DH // 8, 8, CK) + z[None]).reshape(DH, CK).astype(BF16)
        o = _dot(vt, p)
        return o if oacc is None else oacc + o

    def phase(ph, N_, C_, do_qk=True, do_pv=True, pre_qk=None, side=None):
        sN, mN = N_
        sC, mC = C_
        steps = [(t, c) for t in range(UN) for c in range(NC)]
        n = len(steps)
        ws, ms, laccs, ps = {}, {}, {}, {}
        macc = oacc = None
        hist = []
        pv_dep = {}
        cur = (ph, ph // PPB, ph % PPB)
        nxt = (ph + 1, (ph + 1) // PPB, (ph + 1) % PPB)

        def do_exp(i):
            t, c = steps[i]
            if c == 0:
                ms[t] = jnp.broadcast_to(mC[t], (8, TQ))
                laccs[t] = None
            ps[i], laccs[t] = ex_chunk(ms[t], t, c, sC, laccs[t])

        if do_pv:
            for i in range(min(LEAD, n)):
                do_exp(i)
        for i, (t, c) in enumerate(steps):
            if do_qk:
                if c == 0:
                    ws[t] = get_w(nxt, t)
                    macc = None
                z = pre_qk(i, hist) if pre_qk is not None else None
                off = do_pv and (c in OFFC)
                macc = qk_chunk(nxt, t, ws[t](z), c, sN, macc, CK - VR if off else CK)
                hist.append(macc[0:8, 0:128])
                if off:
                    zin = _zero_of(hist[i - LA]) if i >= LA else None
                    sv = qk_vpu(nxt, t, c, sN, zin)
                    macc = jnp.maximum(macc, sv)
                    pv_dep[i + LB] = _zero_of(sv[0:8, 0:128] + sv[8:16, 128:256])
                if c == NC - 1:
                    mN[t] = jnp.max(macc, axis=0, keepdims=True)
            if side is not None:
                side(i)
            if do_pv:
                if i + LEAD < n:
                    do_exp(i + LEAD)
                if c == 0:
                    oacc = None
                oacc = pv_chunk(cur, t, c, ps.pop(i), oacc, pv_dep.get(i))
                if c == NC - 1:
                    head = cur[2] * UN + t
                    ot_s[head] = oacc
                    ls_s[head] = jnp.sum(laccs[t], axis=0, keepdims=True)

    A = (sA, mA)
    B = (sB, mB)

    def ssm_params():
        row1 = lambda ref: ref[...].astype(F32).reshape(1, DM)
        lam_re = row1(lre_ref)
        lam_im = row1(lim_ref)
        dt = jnp.exp(row1(ldt_ref)).astype(BF16).astype(F32)
        mag = jnp.exp(dt * lam_re)
        ang = dt * lam_im
        lb_re = mag * jnp.cos(ang)
        lb_im = mag * jnp.sin(ang)
        den = lam_re * lam_re + lam_im * lam_im
        nre = lb_re - 1.0
        par_s[0] = lb_re
        par_s[1] = lb_im
        par_s[2] = (nre * lam_re + lb_im * lam_im) / den
        par_s[3] = (lb_im * lam_re - nre * lam_im) / den

    def c_rows(r0, r1):
        co_re, co_im = par_s[2], par_s[3]
        cre = cre_s[r0:r1, :].astype(F32)
        cim = cim_s[r0:r1, :].astype(F32)
        a = 2.0 * (cre * co_re - cim * co_im)
        b = -2.0 * (cre * co_im + cim * co_re)
        cp_s[r0:r1, 0:DM] = a.astype(BF16)
        cp_s[r0:r1, DM:2 * DM] = b.astype(BF16)
        return a[0:8, 0:128]

    def scan_step(s, st, ar, ai, store):
        st = list(st)
        for lt in range(NLT):
            hr, hi = st[lt], st[NLT + lt]
            ur = u_s[lt, pl.ds(s, NCHUNK, stride=CLEN), :]
            ui = u_s[NLT + lt, pl.ds(s, NCHUNK, stride=CLEN), :]
            nr = ar[lt] * hr - ai[lt] * hi + ur
            ni = ar[lt] * hi + ai[lt] * hr + ui
            if store:
                u_s[lt, pl.ds(s, NCHUNK, stride=CLEN), :] = nr
                u_s[NLT + lt, pl.ds(s, NCHUNK, stride=CLEN), :] = ni
            st[lt], st[NLT + lt] = nr, ni
        return tuple(st)

    def chunk_carry(ends, ar, ai):
        row = jax.lax.broadcasted_iota(jnp.int32, (NCHUNK, 128), 0)
        init = []
        for lt in range(NLT):
            br, bi = ar[lt], ai[lt]
            pr = pi = None
            e = CLEN
            while e:
                if e & 1:
                    pr, pi = (br, bi) if pr is None else _cmul(pr, pi, br, bi)
                e >>= 1
                if e:
                    br, bi = _cmul(br, bi, br, bi)
            hr = jnp.where(row >= 1, pltpu.roll(ends[lt], 1, 0), 0.0)
            hi = jnp.where(row >= 1, pltpu.roll(ends[NLT + lt], 1, 0), 0.0)
            sh = 1
            while sh < NCHUNK:
                sr = jnp.where(row >= sh, pltpu.roll(hr, sh, 0), 0.0)
                si = jnp.where(row >= sh, pltpu.roll(hi, sh, 0), 0.0)
                dr, di = _cmul(pr, pi, sr, si)
                hr, hi = hr + dr, hi + di
                pr, pi = _cmul(pr, pi, pr, pi)
                sh *= 2
            init.append((hr, hi))
        return tuple(h[0] for h in init) + tuple(h[1] for h in init)

    class PacedScan:
        def __init__(self, nslices):
            lb_re, lb_im = par_s[0], par_s[1]
            tile = lambda v, lt: jnp.broadcast_to(v[:, lt * 128:(lt + 1) * 128], (NCHUNK, 128))
            self.ar = [tile(lb_re, lt) for lt in range(NLT)]
            self.ai = [tile(lb_im, lt) for lt in range(NLT)]
            self.st = tuple(jnp.zeros((NCHUNK, 128), F32) for _ in range(2 * NLT))
            self.items = [(False, s) for s in range(CLEN)] + [None] + [(True, s) for s in range(CLEN)]
            self.n = nslices
            self.crows = {(k * nslices) // (DM // 32): k for k in range(DM // 32)}

        def __call__(self, i, hist):
            lo = (i * len(self.items)) // self.n
            hi = ((i + 1) * len(self.items)) // self.n
            if i >= LAG:
                zin = _zero_of(hist[i - LAG])
                self.st = tuple(h + zin for h in self.st[:NLT]) + tuple(self.st[NLT:])
            for it in self.items[lo:hi]:
                if it is None:
                    self.st = chunk_carry(self.st, self.ar, self.ai)
                else:
                    self.st = scan_step(it[1], self.st, self.ar, self.ai, it[0])
            dep = (self.st[0] + self.st[1]) + (self.st[2] + self.st[3])
            if i in self.crows:
                k = self.crows[i]
                dep = dep + c_rows(32 * k, 32 * (k + 1))
            return _zero_of(dep)

    def proj_ssm_half(i, b_s, lt0):
        r0 = pl.multiple_of(i * TQ, TQ)
        u = _dot(xb_s[pl.ds(r0, TQ), :], b_s[...], _NT)
        for lt in range(NLT):
            u_s[lt0 + lt, pl.ds(r0, TQ), :] = u[:, lt * 128:(lt + 1) * 128]

    def proj_ssm_block(i):
        proj_ssm_half(i, bre_s, 0)
        proj_ssm_half(i, bim_s, NLT)

    def proj_attn_block(i):
        r0 = pl.multiple_of(i * TQ, TQ)
        xc = x_s[pl.ds(r0, TQ), :]
        q = _dot(wt_s[0], xc, _NT).astype(BF16)
        qt = (q.astype(F32) * QSCALE).astype(BF16)
        qt_s[i] = qt
        for hq in range(PPB):
            qf_s[i * PPB + hq] = qt[hq * UN * DH:(hq + 1) * UN * DH, :].astype(F32)
        vt_s[i] = _dot(wt_s[1], xc, _NT).astype(BF16)
        k = _dot(xc, w_s[1]).astype(BF16)
        for p in range(NHEAD // KG):
            kp_s[p, pl.ds(r0, TQ), :] = k[:, DH * KG * p:DH * KG * (p + 1)]
        for cc in range(TQ // CK):
            kr = k[(cc + 1) * CK - VR:(cc + 1) * CK, :].astype(F32)
            row = pl.multiple_of((i * (TQ // CK) + cc) * VR, VR)
            for lt in range(NLT):
                kf_s[lt, pl.ds(row, VR), :] = kr[:, lt * 128:(lt + 1) * 128]

    NPAIR = NQB // PU

    @pl.when(j == 0)
    def _prologue():
        copy(S_BRE).start()
        xb_copy(0).start()
        ssm_params()
        copy(S_BIM).start()
        xb_copy(1).start()
        for lt in range(2 * NLT):
            u_s[lt, SEQ:UROWS, :] = jnp.zeros((UROWS - SEQ, 128), F32)
        copy(S_BRE).wait()
        xb_copy(0).wait()
        proj_ssm_half(0, bre_s, 0)
        copy(S_BIM).wait()
        for r in range(PU, NQB):
            xb_copy(r).start()
        proj_ssm_half(0, bim_s, NLT)
        xb_copy(1).wait()
        proj_ssm_block(1)

        def proj_ssm(i, carry):
            for u in range(PU):
                xb_copy(i * PU + u).wait()

            @pl.when(i == 1)
            def _():
                for k in (S_WQ, S_WV, S_WK):
                    copy(k).start()
                for r in range(NQB):
                    x_copy(r).start()

            for u in range(PU):
                proj_ssm_block(i * PU + u)
            return carry
        jax.lax.fori_loop(1, NPAIR - 1, proj_ssm, 0)

        for u in range(PU):
            xb_copy(NQB - PU + u).wait()
        copy(S_WQ).wait()
        copy(S_WV).wait()
        for k in (S_CRE, S_CIM, S_WO):
            copy(k).start()
        for u in range(PU):
            proj_ssm_block(NQB - PU + u)
            wt_s[u] = w_s[2 * u].T
        copy(S_WK).wait()

        def proj_attn(i, carry):
            for u in range(PA):
                x_copy(i * PA + u).wait()
            for u in range(PA):
                proj_attn_block(i * PA + u)
            return carry
        jax.lax.fori_loop(0, NQB // PA, proj_attn, 0)

        for k in (S_CRE, S_CIM, S_WO):
            copy(k).wait()

    @pl.when(j == 0)
    def _fill():
        phase(-1, A, B, do_pv=False, pre_qk=PacedScan(UN * NC))

    nph = jnp.where(j == NQB - 1, PPB - 1, PPB)

    def phase_pair(i, carry):
        ph = j * PPB + 2 * i
        phase(ph, B, A)

        @pl.when(2 * i + 1 < nph)
        def _odd():
            phase(ph + 1, A, B)
        return carry

    jax.lax.fori_loop(0, PPB // 2, phase_pair, 0)

    slot = j % 2

    @pl.when(j >= 2)
    def _free_slot():
        out_copy(j - 2, 0).wait()
        out_copy(j - 2, 1).wait()

    def ssm_out():
        r0 = pl.multiple_of(j * TQ, TQ)
        g = jnp.concatenate([u_s[lt, pl.ds(r0, TQ), :] for lt in range(2 * NLT)], axis=1).astype(BF16)
        y = _dot(g, cp_s[...], _NT)
        d = dsk_ref[...].astype(F32).reshape(1, DM)
        o_s[slot, :, DM:2 * DM] = y + xb_s[pl.ds(r0, TQ), :].astype(F32) * d

    def attn_out():
        o = (ot_s[...] * (1.0 / ls_s[...])).reshape(DM, TQ).astype(BF16)
        o_s[slot, :, 0:DM] = _dot(o, wo_s[...], _TN)

    class SsmOutPieces:
        def __init__(self, nsteps):
            self.r0 = (NQB - 1) * TQ
            self.npieces = NLT * 2 * NLT
            self.at = {(p * nsteps) // self.npieces: p for p in range(self.npieces)}
            self.acc = None

        def __call__(self, i):
            if i not in self.at:
                return
            n, k = divmod(self.at[i], 2 * NLT)
            g = u_s[k, self.r0:self.r0 + TQ, :].astype(BF16)
            part = _dot(g, cp_s[n * 128:(n + 1) * 128, k * 128:(k + 1) * 128], _NT)
            self.acc = part if k == 0 else self.acc + part
            if k == 2 * NLT - 1:
                d = dsk_ref[...].astype(F32).reshape(1, DM)[:, n * 128:(n + 1) * 128]
                xb = xb_s[self.r0:self.r0 + TQ, n * 128:(n + 1) * 128].astype(F32)
                o_s[(NQB - 1) % 2, :, DM + n * 128:DM + (n + 1) * 128] = self.acc + xb * d

    @pl.when(j < NQB - 1)
    def _notlast():
        ssm_out()
        attn_out()
        out_copy(j, 0).start()
        out_copy(j, 1).start()

    @pl.when(j == NQB - 1)
    def _last():
        phase(NPH - 1, A, B, do_qk=False, side=SsmOutPieces(UN * NC))
        out_copy(j, 1).start()

    @pl.when(j == NQB - 1)
    def _last2():
        attn_out()
        out_copy(j, 0).start()
        out_copy(j - 1, 0).wait()
        out_copy(j - 1, 1).wait()
        out_copy(j, 1).wait()
        out_copy(j, 0).wait()


@jax.jit
def pallas_concat_heads__softmax_full_mha__ssm_conv_s5__prompt_kernel(
    A_x, A_wqkv, A_wo, B_x, B_Lambda_re, B_Lambda_im, B_B_re, B_B_im, B_C_re, B_C_im,
    B_log_dt, B_Dskip,
):
    hbm = pl.BlockSpec(memory_space=pl.ANY)
    vec = pl.BlockSpec((DM,), lambda j: (0,))
    args = (A_x.reshape(SEQ, DM), A_wqkv, A_wo, B_x.reshape(SEQ, DM), B_Lambda_re,
            B_Lambda_im, B_B_re, B_B_im, B_C_re, B_C_im, B_log_dt, B_Dskip)
    in_specs = [hbm, hbm, hbm, hbm, vec, vec, hbm, hbm, hbm, hbm, vec, vec]
    scratch = [
        pltpu.VMEM((SEQ, DM), BF16),
        pltpu.VMEM((3, DM, DM), BF16),
        pltpu.VMEM((DM, DM), BF16),
        pltpu.VMEM((SEQ, DM), BF16),
        pltpu.VMEM((DM, DM), BF16),
        pltpu.VMEM((DM, DM), BF16),
        pltpu.VMEM((DM, DM), BF16),
        pltpu.VMEM((DM, DM), BF16),
        pltpu.VMEM((2, TQ, 2 * DM), F32),
        pltpu.SemaphoreType.DMA((NSEM,)),
        pltpu.VMEM((2, DM, DM), BF16),
        pltpu.VMEM((NQB, DM, TQ), BF16),
        pltpu.VMEM((NQB, DM, TQ), BF16),
        pltpu.VMEM((NHEAD // KG, SEQ, DH * KG), BF16),
        pltpu.VMEM((UN, SEQ, TQ), F32),
        pltpu.VMEM((UN, SEQ, TQ), F32),
        pltpu.VMEM((UN, 1, TQ), F32),
        pltpu.VMEM((UN, 1, TQ), F32),
        pltpu.VMEM((NHEAD, DH, TQ), F32),
        pltpu.VMEM((NHEAD, 1, TQ), F32),
        pltpu.VMEM((2 * NLT, UROWS, 128), F32),
        pltpu.VMEM((DM, 2 * DM), BF16),
        pltpu.VMEM((NLT, NC * VR, 128), F32),
        pltpu.VMEM((NPH, UN * DH, TQ), F32),
        pltpu.VMEM((4, 1, DM), F32),
    ]
    out = pl.pallas_call(
        _kernel,
        grid=(NQB,),
        in_specs=in_specs,
        out_specs=pl.BlockSpec(memory_space=pl.ANY),
        out_shape=jax.ShapeDtypeStruct((SEQ, 2 * DM), F32),
        scratch_shapes=scratch,
        compiler_params=pltpu.CompilerParams(
            dimension_semantics=("arbitrary",),
            vmem_limit_bytes=110 * 1024 * 1024),
    )(*args)
    return out.reshape(1, SEQ, 2 * DM)
```

```python
import math

import jax
import jax.numpy as jnp
import jax.experimental.pallas as pl
import jax.experimental.pallas.tpu as pltpu

F32 = jnp.float32
BF16 = jnp.bfloat16

SEQ = 2048
DM = 512
NHEAD = 32
DH = 16
TQ = 256
NQB = SEQ // TQ
UN = 8
PPB = NHEAD // UN
NPH = NQB * PPB
CK = 128
NC = SEQ // CK
NACC = 2
KG = 4
LEAD = 2
VR = 16
OFFC = (1, 3, 6, 8, 11, 13)
LA = 3
LB = 9
LAG = 6
CROWS = 8
PU = 2
PA = 4
NCHUNK = 8
CLEN = SEQ // NCHUNK + 1
UROWS = NCHUNK * CLEN
NLT = DM // 128
QSCALE = (DH ** -0.5) * math.log2(math.e)

_NN = (((1,), (0,)), ((), ()))
_NT = (((1,), (1,)), ((), ()))
_TN = (((0,), (0,)), ((), ()))

S_WQ, S_WK, S_WV, S_BRE, S_BIM, S_CRE, S_CIM, S_WO, S_X0 = range(9)
S_XB0 = S_X0 + NQB
S_OUT = S_XB0 + NQB
NSEM = S_OUT + 4


def _dot(a, b, dims=_NN):
    return jax.lax.dot_general(a, b, dims, preferred_element_type=F32)


def _red(x, op):
    r = x.shape[0]
    return op(x.reshape(r // (8 * NACC), 8 * NACC, x.shape[1]), axis=0)


def _zero_of(v):
    i = v.astype(jnp.int32)
    i = jax.lax.shift_right_logical(jax.lax.shift_right_logical(i, 31), 1)
    return i.astype(F32)


def _cmul(ar, ai, br, bi):
    return ar * br - ai * bi, ar * bi + ai * br


def _kernel(x_hbm, wqkv_hbm, wo_hbm, xb_hbm, lre_ref, lim_ref, bre_hbm, bim_hbm,
            cre_hbm, cim_hbm, ldt_ref, dsk_ref,
            o_hbm,
            x_s, w_s, wo_s, xb_s, bre_s, bim_s, cre_s, cim_s, o_s, sems,
            wt_s, qt_s, vt_s, kp_s, sA, sB, mA, mB, ot_s, ls_s, u_s, cp_s, kf_s, qf_s, par_s):
    j = pl.program_id(0)

    def rows_copy(src, dst, i, sem0):
        rows = pl.ds(pl.multiple_of(i * TQ, TQ), TQ)
        return pltpu.make_async_copy(src.at[rows], dst.at[rows], sems.at[sem0 + i])

    x_copy = lambda i: rows_copy(x_hbm, x_s, i, S_X0)
    xb_copy = lambda i: rows_copy(xb_hbm, xb_s, i, S_XB0)

    whole = {
        S_WQ: (wqkv_hbm.at[:, 0:DM], w_s.at[0]), S_WK: (wqkv_hbm.at[:, DM:2 * DM], w_s.at[1]),
        S_WV: (wqkv_hbm.at[:, 2 * DM:3 * DM], w_s.at[2]),
        S_BRE: (bre_hbm, bre_s), S_BIM: (bim_hbm, bim_s),
        S_CRE: (cre_hbm, cre_s), S_CIM: (cim_hbm, cim_s), S_WO: (wo_hbm, wo_s),
    }

    def copy(k):
        src, dst = whole[k]
        return pltpu.make_async_copy(src, dst, sems.at[k])

    def out_copy(step, half):
        slot = step % 2
        rows = pl.ds(pl.multiple_of(step * TQ, TQ), TQ)
        cols = pl.ds(half * DM, DM)
        return pltpu.make_async_copy(o_s.at[slot, :, cols], o_hbm.at[rows, cols],
                                     sems.at[S_OUT + 2 * slot + half])

    def head_rows(head):
        return pl.ds(pl.multiple_of(head * DH, DH), DH)

    def get_w(grp, t):
        _, qb, hq = grp
        q = qt_s[qb, head_rows(hq * UN + t), :]

        def pad(q):
            parts = [jnp.zeros((DH, TQ), BF16)] * KG
            parts[t % KG] = q
            return jnp.concatenate(parts, axis=0)

        w0 = pad(q)

        def make(z):
            if z is None:
                return w0
            zz = jnp.concatenate([z] * (TQ // 128), axis=1)[None]
            qz = q.astype(F32).reshape(DH // 8, 8, TQ) + zz
            return pad(qz.reshape(DH, TQ).astype(BF16))
        return make

    def qk_chunk(grp, t, w, c, s_ref, macc, nrows):
        karr = grp[2] * (UN // KG) + t // KG
        s = _dot(kp_s[karr, c * CK:c * CK + nrows, :], w)
        s_ref[t, c * CK:c * CK + nrows, :] = s
        if nrows == CK:
            r = _red(s, jnp.max)
        else:
            r = jnp.max(s.reshape(nrows // VR, VR, TQ), axis=0)
        return r if macc is None else jnp.maximum(macc, r)

    def qk_vpu(grp, t, c, s_ref, zin):
        g, _, hq = grp
        kf = kf_s[hq, c * VR:(c + 1) * VR, :]
        if zin is not None:
            kf = (kf.reshape(VR // 8, 8, 128) + zin[None]).reshape(VR, 128)
        s = None
        for d in range(DH):
            col = t * DH + d
            qb = jnp.concatenate(
                [jnp.broadcast_to(qf_s[g, col:col + 1, qt * 128:(qt + 1) * 128], (8, 128))
                 for qt in range(TQ // 128)], axis=1)
            kb = jnp.broadcast_to(kf[:, col:col + 1], (VR, TQ)).reshape(VR // 8, 8, TQ)
            p = kb * qb[None]
            s = p if s is None else s + p
        s = s.reshape(VR, TQ)
        s_ref[t, (c + 1) * CK - VR:(c + 1) * CK, :] = s
        return s

    def ex_chunk(m, t, c, s_ref, lacc):
        s = s_ref[t, c * CK:(c + 1) * CK, :].reshape(CK // 8, 8, TQ)
        p = jnp.exp2(s - m[None]).reshape(CK, TQ)
        r = _red(p, jnp.sum)
        return p.astype(BF16), (r if lacc is None else lacc + r)

    def pv_chunk(grp, t, c, p, oacc, z):
        k0 = c * CK
        vt = vt_s[k0 // TQ, head_rows(grp[2] * UN + t), k0 % TQ:k0 % TQ + CK]
        if z is not None:
            vt = (vt.astype(F32).reshape(DH // 8, 8, CK) + z[None]).reshape(DH, CK).astype(BF16)
        o = _dot(vt, p)
        return o if oacc is None else oacc + o

    def phase(ph, N_, C_, do_qk=True, do_pv=True, pre_qk=None, side=None):
        sN, mN = N_
        sC, mC = C_
        steps = [(t, c) for t in range(UN) for c in range(NC)]
        n = len(steps)
        ws, ms, laccs, ps = {}, {}, {}, {}
        macc = oacc = None
        hist = []
        pv_dep = {}
        cur = (ph, ph // PPB, ph % PPB)
        nxt = (ph + 1, (ph + 1) // PPB, (ph + 1) % PPB)

        def do_exp(i):
            t, c = steps[i]
            if c == 0:
                ms[t] = jnp.broadcast_to(mC[t], (8, TQ))
                laccs[t] = None
            ps[i], laccs[t] = ex_chunk(ms[t], t, c, sC, laccs[t])

        if do_pv:
            for i in range(min(LEAD, n)):
                do_exp(i)
        for i, (t, c) in enumerate(steps):
            if do_qk:
                if c == 0:
                    ws[t] = get_w(nxt, t)
                    macc = None
                z = pre_qk(i, hist) if pre_qk is not None else None
                off = do_pv and (c in OFFC)
                macc = qk_chunk(nxt, t, ws[t](z), c, sN, macc, CK - VR if off else CK)
                hist.append(macc[0:8, 0:128])
                if off:
                    zin = _zero_of(hist[i - LA]) if i >= LA else None
                    sv = qk_vpu(nxt, t, c, sN, zin)
                    macc = jnp.maximum(macc, sv)
                    pv_dep[i + LB] = _zero_of(sv[0:8, 0:128] + sv[8:16, 128:256])
                if c == NC - 1:
                    mN[t] = jnp.max(macc, axis=0, keepdims=True)
            if side is not None:
                side(i)
            if do_pv:
                if i + LEAD < n:
                    do_exp(i + LEAD)
                if c == 0:
                    oacc = None
                oacc = pv_chunk(cur, t, c, ps.pop(i), oacc, pv_dep.get(i))
                if c == NC - 1:
                    head = cur[2] * UN + t
                    ot_s[head] = oacc
                    ls_s[head] = jnp.sum(laccs[t], axis=0, keepdims=True)

    A = (sA, mA)
    B = (sB, mB)

    def ssm_params():
        row1 = lambda ref: ref[...].astype(F32).reshape(1, DM)
        lam_re = row1(lre_ref)
        lam_im = row1(lim_ref)
        dt = jnp.exp(row1(ldt_ref)).astype(BF16).astype(F32)
        mag = jnp.exp(dt * lam_re)
        ang = dt * lam_im
        lb_re = mag * jnp.cos(ang)
        lb_im = mag * jnp.sin(ang)
        den = lam_re * lam_re + lam_im * lam_im
        nre = lb_re - 1.0
        par_s[0] = lb_re
        par_s[1] = lb_im
        par_s[2] = (nre * lam_re + lb_im * lam_im) / den
        par_s[3] = (lb_im * lam_re - nre * lam_im) / den

    def c_rows(r0, r1):
        co_re, co_im = par_s[2], par_s[3]
        cre = cre_s[r0:r1, :].astype(F32)
        cim = cim_s[r0:r1, :].astype(F32)
        a = 2.0 * (cre * co_re - cim * co_im)
        b = -2.0 * (cre * co_im + cim * co_re)
        cp_s[r0:r1, 0:DM] = a.astype(BF16)
        cp_s[r0:r1, DM:2 * DM] = b.astype(BF16)
        return a[0:8, 0:128]

    def scan_step(s, st, ar, ai, store):
        st = list(st)
        for lt in range(NLT):
            hr, hi = st[lt], st[NLT + lt]
            ur = u_s[lt, pl.ds(s, NCHUNK, stride=CLEN), :]
            ui = u_s[NLT + lt, pl.ds(s, NCHUNK, stride=CLEN), :]
            nr = ar[lt] * hr - ai[lt] * hi + ur
            ni = ar[lt] * hi + ai[lt] * hr + ui
            if store:
                u_s[lt, pl.ds(s, NCHUNK, stride=CLEN), :] = nr
                u_s[NLT + lt, pl.ds(s, NCHUNK, stride=CLEN), :] = ni
            st[lt], st[NLT + lt] = nr, ni
        return tuple(st)

    def chunk_carry(ends, ar, ai):
        row = jax.lax.broadcasted_iota(jnp.int32, (NCHUNK, 128), 0)
        init = []
        for lt in range(NLT):
            br, bi = ar[lt], ai[lt]
            pr = pi = None
            e = CLEN
            while e:
                if e & 1:
                    pr, pi = (br, bi) if pr is None else _cmul(pr, pi, br, bi)
                e >>= 1
                if e:
                    br, bi = _cmul(br, bi, br, bi)
            hr = jnp.where(row >= 1, pltpu.roll(ends[lt], 1, 0), 0.0)
            hi = jnp.where(row >= 1, pltpu.roll(ends[NLT + lt], 1, 0), 0.0)
            sh = 1
            while sh < NCHUNK:
                sr = jnp.where(row >= sh, pltpu.roll(hr, sh, 0), 0.0)
                si = jnp.where(row >= sh, pltpu.roll(hi, sh, 0), 0.0)
                dr, di = _cmul(pr, pi, sr, si)
                hr, hi = hr + dr, hi + di
                pr, pi = _cmul(pr, pi, pr, pi)
                sh *= 2
            init.append((hr, hi))
        return tuple(h[0] for h in init) + tuple(h[1] for h in init)

    class PacedScan:
        def __init__(self, nslices):
            lb_re, lb_im = par_s[0], par_s[1]
            tile = lambda v, lt: jnp.broadcast_to(v[:, lt * 128:(lt + 1) * 128], (NCHUNK, 128))
            self.ar = [tile(lb_re, lt) for lt in range(NLT)]
            self.ai = [tile(lb_im, lt) for lt in range(NLT)]
            self.st = tuple(jnp.zeros((NCHUNK, 128), F32) for _ in range(2 * NLT))
            self.items = [(False, s) for s in range(CLEN)] + [None] + [(True, s) for s in range(CLEN)]
            self.n = nslices
            self.crows = {(k * nslices) // (DM // CROWS): k for k in range(DM // CROWS)}

        def __call__(self, i, hist):
            lo = (i * len(self.items)) // self.n
            hi = ((i + 1) * len(self.items)) // self.n
            if i >= LAG:
                zin = _zero_of(hist[i - LAG])
                self.st = tuple(h + zin for h in self.st[:NLT]) + tuple(self.st[NLT:])
            for it in self.items[lo:hi]:
                if it is None:
                    self.st = chunk_carry(self.st, self.ar, self.ai)
                else:
                    self.st = scan_step(it[1], self.st, self.ar, self.ai, it[0])
            dep = (self.st[0] + self.st[1]) + (self.st[2] + self.st[3])
            if i in self.crows:
                k = self.crows[i]
                dep = dep + c_rows(CROWS * k, CROWS * (k + 1))
            return _zero_of(dep)

    def proj_ssm_half(i, b_s, lt0):
        r0 = pl.multiple_of(i * TQ, TQ)
        u = _dot(xb_s[pl.ds(r0, TQ), :], b_s[...], _NT)
        for lt in range(NLT):
            u_s[lt0 + lt, pl.ds(r0, TQ), :] = u[:, lt * 128:(lt + 1) * 128]

    def proj_ssm_block(i):
        proj_ssm_half(i, bre_s, 0)
        proj_ssm_half(i, bim_s, NLT)

    def proj_attn_block(i):
        r0 = pl.multiple_of(i * TQ, TQ)
        xc = x_s[pl.ds(r0, TQ), :]
        q = _dot(wt_s[0], xc, _NT).astype(BF16)
        qt = (q.astype(F32) * QSCALE).astype(BF16)
        qt_s[i] = qt
        for hq in range(PPB):
            qf_s[i * PPB + hq] = qt[hq * UN * DH:(hq + 1) * UN * DH, :].astype(F32)
        vt_s[i] = _dot(wt_s[1], xc, _NT).astype(BF16)
        k = _dot(xc, w_s[1]).astype(BF16)
        for p in range(NHEAD // KG):
            kp_s[p, pl.ds(r0, TQ), :] = k[:, DH * KG * p:DH * KG * (p + 1)]
        for cc in range(TQ // CK):
            kr = k[(cc + 1) * CK - VR:(cc + 1) * CK, :].astype(F32)
            row = pl.multiple_of((i * (TQ // CK) + cc) * VR, VR)
            for lt in range(NLT):
                kf_s[lt, pl.ds(row, VR), :] = kr[:, lt * 128:(lt + 1) * 128]

    NPAIR = NQB // PU

    @pl.when(j == 0)
    def _prologue():
        copy(S_BRE).start()
        xb_copy(0).start()
        ssm_params()
        copy(S_BIM).start()
        xb_copy(1).start()
        for lt in range(2 * NLT):
            u_s[lt, SEQ:UROWS, :] = jnp.zeros((UROWS - SEQ, 128), F32)
        copy(S_BRE).wait()
        xb_copy(0).wait()
        proj_ssm_half(0, bre_s, 0)
        copy(S_BIM).wait()
        for r in range(PU, NQB):
            xb_copy(r).start()
        proj_ssm_half(0, bim_s, NLT)
        xb_copy(1).wait()
        proj_ssm_block(1)

        def proj_ssm(i, carry):
            for u in range(PU):
                xb_copy(i * PU + u).wait()

            @pl.when(i == 1)
            def _():
                for k in (S_WQ, S_WV, S_WK):
                    copy(k).start()
                for r in range(NQB):
                    x_copy(r).start()

            for u in range(PU):
                proj_ssm_block(i * PU + u)
            return carry
        jax.lax.fori_loop(1, NPAIR - 1, proj_ssm, 0)

        for u in range(PU):
            xb_copy(NQB - PU + u).wait()
        copy(S_WQ).wait()
        copy(S_WV).wait()
        for k in (S_CRE, S_CIM, S_WO):
            copy(k).start()
        for u in range(PU):
            proj_ssm_block(NQB - PU + u)
            wt_s[u] = w_s[2 * u].T
        copy(S_WK).wait()

        def proj_attn(i, carry):
            for u in range(PA):
                x_copy(i * PA + u).wait()
            for u in range(PA):
                proj_attn_block(i * PA + u)
            return carry
        jax.lax.fori_loop(0, NQB // PA, proj_attn, 0)

        for k in (S_CRE, S_CIM, S_WO):
            copy(k).wait()

    @pl.when(j == 0)
    def _fill():
        phase(-1, A, B, do_pv=False, pre_qk=PacedScan(UN * NC))

    nph = jnp.where(j == NQB - 1, PPB - 1, PPB)

    def phase_pair(i, carry):
        ph = j * PPB + 2 * i
        phase(ph, B, A)

        @pl.when(2 * i + 1 < nph)
        def _odd():
            phase(ph + 1, A, B)
        return carry

    jax.lax.fori_loop(0, PPB // 2, phase_pair, 0)

    slot = j % 2

    @pl.when(j >= 2)
    def _free_slot():
        out_copy(j - 2, 0).wait()
        out_copy(j - 2, 1).wait()

    def ssm_out():
        r0 = pl.multiple_of(j * TQ, TQ)
        g = jnp.concatenate([u_s[lt, pl.ds(r0, TQ), :] for lt in range(2 * NLT)], axis=1).astype(BF16)
        y = _dot(g, cp_s[...], _NT)
        d = dsk_ref[...].astype(F32).reshape(1, DM)
        o_s[slot, :, DM:2 * DM] = y + xb_s[pl.ds(r0, TQ), :].astype(F32) * d

    def attn_out():
        o = (ot_s[...] * (1.0 / ls_s[...])).reshape(DM, TQ).astype(BF16)
        o_s[slot, :, 0:DM] = _dot(o, wo_s[...], _TN)

    class SsmOutPieces:
        def __init__(self, nsteps):
            self.r0 = (NQB - 1) * TQ
            self.npieces = NLT * 2 * NLT
            self.at = {(p * nsteps) // self.npieces: p for p in range(self.npieces)}
            self.acc = None

        def __call__(self, i):
            if i not in self.at:
                return
            n, k = divmod(self.at[i], 2 * NLT)
            g = u_s[k, self.r0:self.r0 + TQ, :].astype(BF16)
            part = _dot(g, cp_s[n * 128:(n + 1) * 128, k * 128:(k + 1) * 128], _NT)
            self.acc = part if k == 0 else self.acc + part
            if k == 2 * NLT - 1:
                d = dsk_ref[...].astype(F32).reshape(1, DM)[:, n * 128:(n + 1) * 128]
                xb = xb_s[self.r0:self.r0 + TQ, n * 128:(n + 1) * 128].astype(F32)
                o_s[(NQB - 1) % 2, :, DM + n * 128:DM + (n + 1) * 128] = self.acc + xb * d

    @pl.when(j < NQB - 1)
    def _notlast():
        ssm_out()
        attn_out()
        out_copy(j, 0).start()
        out_copy(j, 1).start()

    @pl.when(j == NQB - 1)
    def _last():
        phase(NPH - 1, A, B, do_qk=False, side=SsmOutPieces(UN * NC))
        out_copy(j, 1).start()

    @pl.when(j == NQB - 1)
    def _last2():
        attn_out()
        out_copy(j, 0).start()
        out_copy(j - 1, 0).wait()
        out_copy(j - 1, 1).wait()
        out_copy(j, 1).wait()
        out_copy(j, 0).wait()


@jax.jit
def pallas_concat_heads__softmax_full_mha__ssm_conv_s5__prompt_kernel(
    A_x, A_wqkv, A_wo, B_x, B_Lambda_re, B_Lambda_im, B_B_re, B_B_im, B_C_re, B_C_im,
    B_log_dt, B_Dskip,
):
    hbm = pl.BlockSpec(memory_space=pl.ANY)
    vec = pl.BlockSpec((DM,), lambda j: (0,))
    args = (A_x.reshape(SEQ, DM), A_wqkv, A_wo, B_x.reshape(SEQ, DM), B_Lambda_re,
            B_Lambda_im, B_B_re, B_B_im, B_C_re, B_C_im, B_log_dt, B_Dskip)
    in_specs = [hbm, hbm, hbm, hbm, vec, vec, hbm, hbm, hbm, hbm, vec, vec]
    scratch = [
        pltpu.VMEM((SEQ, DM), BF16),
        pltpu.VMEM((3, DM, DM), BF16),
        pltpu.VMEM((DM, DM), BF16),
        pltpu.VMEM((SEQ, DM), BF16),
        pltpu.VMEM((DM, DM), BF16),
        pltpu.VMEM((DM, DM), BF16),
        pltpu.VMEM((DM, DM), BF16),
        pltpu.VMEM((DM, DM), BF16),
        pltpu.VMEM((2, TQ, 2 * DM), F32),
        pltpu.SemaphoreType.DMA((NSEM,)),
        pltpu.VMEM((2, DM, DM), BF16),
        pltpu.VMEM((NQB, DM, TQ), BF16),
        pltpu.VMEM((NQB, DM, TQ), BF16),
        pltpu.VMEM((NHEAD // KG, SEQ, DH * KG), BF16),
        pltpu.VMEM((UN, SEQ, TQ), F32),
        pltpu.VMEM((UN, SEQ, TQ), F32),
        pltpu.VMEM((UN, 1, TQ), F32),
        pltpu.VMEM((UN, 1, TQ), F32),
        pltpu.VMEM((NHEAD, DH, TQ), F32),
        pltpu.VMEM((NHEAD, 1, TQ), F32),
        pltpu.VMEM((2 * NLT, UROWS, 128), F32),
        pltpu.VMEM((DM, 2 * DM), BF16),
        pltpu.VMEM((NLT, NC * VR, 128), F32),
        pltpu.VMEM((NPH, UN * DH, TQ), F32),
        pltpu.VMEM((4, 1, DM), F32),
    ]
    out = pl.pallas_call(
        _kernel,
        grid=(NQB,),
        in_specs=in_specs,
        out_specs=pl.BlockSpec(memory_space=pl.ANY),
        out_shape=jax.ShapeDtypeStruct((SEQ, 2 * DM), F32),
        scratch_shapes=scratch,
        compiler_params=pltpu.CompilerParams(
            dimension_semantics=("arbitrary",),
            vmem_limit_bytes=110 * 1024 * 1024),
    )(*args)
    return out.reshape(1, SEQ, 2 * DM)
```

```python
import math

import jax
import jax.numpy as jnp
import jax.experimental.pallas as pl
import jax.experimental.pallas.tpu as pltpu

F32 = jnp.float32
BF16 = jnp.bfloat16

SEQ = 2048
DM = 512
NHEAD = 32
DH = 16
TQ = 256
NQB = SEQ // TQ
UN = 8
PPB = NHEAD // UN
NPH = NQB * PPB
CK = 128
NC = SEQ // CK
NACC = 2
KG = 4
LEAD = 2
VR = 16
OFFC = (1, 3, 5, 8, 11, 13)
LB = 5
LAG = 6
CROWS = 8
PU = 2
PA = 4
NCHUNK = 8
CLEN = SEQ // NCHUNK + 1
UROWS = NCHUNK * CLEN
NLT = DM // 128
QSCALE = (DH ** -0.5) * math.log2(math.e)

_NN = (((1,), (0,)), ((), ()))
_NT = (((1,), (1,)), ((), ()))
_TN = (((0,), (0,)), ((), ()))

S_WQ, S_WK, S_WV, S_BRE, S_BIM, S_CRE, S_CIM, S_WO, S_X0 = range(9)
S_XB0 = S_X0 + NQB
S_OUT = S_XB0 + NQB
NSEM = S_OUT + 4


def _dot(a, b, dims=_NN):
    return jax.lax.dot_general(a, b, dims, preferred_element_type=F32)


def _red(x, op):
    r = x.shape[0]
    return op(x.reshape(r // (8 * NACC), 8 * NACC, x.shape[1]), axis=0)


def _zero_of(v):
    i = v.astype(jnp.int32)
    i = jax.lax.shift_right_logical(jax.lax.shift_right_logical(i, 31), 1)
    return i.astype(F32)


def _cmul(ar, ai, br, bi):
    return ar * br - ai * bi, ar * bi + ai * br


def _kernel(x_hbm, wqkv_hbm, wo_hbm, xb_hbm, lre_ref, lim_ref, bre_hbm, bim_hbm,
            cre_hbm, cim_hbm, ldt_ref, dsk_ref,
            o_hbm,
            x_s, w_s, wo_s, xb_s, bre_s, bim_s, cre_s, cim_s, o_s, sems,
            wt_s, qt_s, vt_s, kp_s, sA, sB, mA, mB, ot_s, ls_s, u_s, cp_s, kf_s, qf_s, par_s):
    j = pl.program_id(0)

    def rows_copy(src, dst, i, sem0):
        rows = pl.ds(pl.multiple_of(i * TQ, TQ), TQ)
        return pltpu.make_async_copy(src.at[rows], dst.at[rows], sems.at[sem0 + i])

    x_copy = lambda i: rows_copy(x_hbm, x_s, i, S_X0)
    xb_copy = lambda i: rows_copy(xb_hbm, xb_s, i, S_XB0)

    whole = {
        S_WQ: (wqkv_hbm.at[:, 0:DM], w_s.at[0]), S_WK: (wqkv_hbm.at[:, DM:2 * DM], w_s.at[1]),
        S_WV: (wqkv_hbm.at[:, 2 * DM:3 * DM], w_s.at[2]),
        S_BRE: (bre_hbm, bre_s), S_BIM: (bim_hbm, bim_s),
        S_CRE: (cre_hbm, cre_s), S_CIM: (cim_hbm, cim_s), S_WO: (wo_hbm, wo_s),
    }

    def copy(k):
        src, dst = whole[k]
        return pltpu.make_async_copy(src, dst, sems.at[k])

    def out_copy(step, half):
        slot = step % 2
        rows = pl.ds(pl.multiple_of(step * TQ, TQ), TQ)
        cols = pl.ds(half * DM, DM)
        return pltpu.make_async_copy(o_s.at[slot, :, cols], o_hbm.at[rows, cols],
                                     sems.at[S_OUT + 2 * slot + half])

    def head_rows(head):
        return pl.ds(pl.multiple_of(head * DH, DH), DH)

    def get_w(grp, t):
        _, qb, hq = grp
        q = qt_s[qb, head_rows(hq * UN + t), :]

        def pad(q):
            parts = [jnp.zeros((DH, TQ), BF16)] * KG
            parts[t % KG] = q
            return jnp.concatenate(parts, axis=0)

        w0 = pad(q)

        def make(z):
            if z is None:
                return w0
            zz = jnp.concatenate([z] * (TQ // 128), axis=1)[None]
            qz = q.astype(F32).reshape(DH // 8, 8, TQ) + zz
            return pad(qz.reshape(DH, TQ).astype(BF16))
        return make

    def qk_chunk(grp, t, w, c, s_ref, macc, nrows):
        karr = grp[2] * (UN // KG) + t // KG
        s = _dot(kp_s[karr, c * CK:c * CK + nrows, :], w)
        s_ref[t, c * CK:c * CK + nrows, :] = s
        if nrows == CK:
            r = _red(s, jnp.max)
        else:
            r = jnp.max(s.reshape(nrows // VR, VR, TQ), axis=0)
        return r if macc is None else jnp.maximum(macc, r)

    def qk_vpu(grp, t, c, s_ref):
        g, _, hq = grp
        kf = kf_s[hq, c * VR:(c + 1) * VR, :]
        s = None
        for d in range(DH):
            col = t * DH + d
            qb = jnp.concatenate(
                [jnp.broadcast_to(qf_s[g, col:col + 1, qt * 128:(qt + 1) * 128], (8, 128))
                 for qt in range(TQ // 128)], axis=1)
            kb = jnp.broadcast_to(kf[:, col:col + 1], (VR, TQ)).reshape(VR // 8, 8, TQ)
            p = kb * qb[None]
            s = p if s is None else s + p
        s = s.reshape(VR, TQ)
        s_ref[t, (c + 1) * CK - VR:(c + 1) * CK, :] = s
        return s

    def ex_chunk(m, t, c, s_ref, lacc):
        s = s_ref[t, c * CK:(c + 1) * CK, :].reshape(CK // 8, 8, TQ)
        p = jnp.exp2(s - m[None]).reshape(CK, TQ)
        r = _red(p, jnp.sum)
        return p.astype(BF16), (r if lacc is None else lacc + r)

    def pv_chunk(grp, t, c, p, oacc, z):
        k0 = c * CK
        vt = vt_s[k0 // TQ, head_rows(grp[2] * UN + t), k0 % TQ:k0 % TQ + CK]
        if z is not None:
            vt = (vt.astype(F32).reshape(DH // 8, 8, CK) + z[None]).reshape(DH, CK).astype(BF16)
        o = _dot(vt, p)
        return o if oacc is None else oacc + o

    def phase(ph, N_, C_, do_qk=True, do_pv=True, pre_qk=None, side=None):
        sN, mN = N_
        sC, mC = C_
        steps = [(t, c) for t in range(UN) for c in range(NC)]
        n = len(steps)
        ws, ms, laccs, ps = {}, {}, {}, {}
        macc = oacc = None
        hist = []
        pv_dep = {}
        cur = (ph, ph // PPB, ph % PPB)
        nxt = (ph + 1, (ph + 1) // PPB, (ph + 1) % PPB)

        def do_exp(i):
            t, c = steps[i]
            if c == 0:
                ms[t] = jnp.broadcast_to(mC[t], (8, TQ))
                laccs[t] = None
            ps[i], laccs[t] = ex_chunk(ms[t], t, c, sC, laccs[t])

        if do_pv:
            for i in range(min(LEAD, n)):
                do_exp(i)
        for i, (t, c) in enumerate(steps):
            if do_qk:
                if c == 0:
                    ws[t] = get_w(nxt, t)
                    macc = None
                z = pre_qk(i, hist) if pre_qk is not None else None
                off = do_pv and (c in OFFC)
                macc = qk_chunk(nxt, t, ws[t](z), c, sN, macc, CK - VR if off else CK)
                hist.append(macc[0:8, 0:128])
                if off:
                    sv = qk_vpu(nxt, t, c, sN)
                    macc = jnp.maximum(macc, sv)
                    pv_dep[i + LB] = _zero_of(sv[0:8, 0:128] + sv[8:16, 128:256])
                if c == NC - 1:
                    mN[t] = jnp.max(macc, axis=0, keepdims=True)
            if side is not None:
                side(i)
            if do_pv:
                if i + LEAD < n:
                    do_exp(i + LEAD)
                if c == 0:
                    oacc = None
                oacc = pv_chunk(cur, t, c, ps.pop(i), oacc, pv_dep.get(i))
                if c == NC - 1:
                    head = cur[2] * UN + t
                    ot_s[head] = oacc
                    ls_s[head] = jnp.sum(laccs[t], axis=0, keepdims=True)

    A = (sA, mA)
    B = (sB, mB)

    def ssm_params():
        row1 = lambda ref: ref[...].astype(F32).reshape(1, DM)
        lam_re = row1(lre_ref)
        lam_im = row1(lim_ref)
        dt = jnp.exp(row1(ldt_ref)).astype(BF16).astype(F32)
        mag = jnp.exp(dt * lam_re)
        ang = dt * lam_im
        lb_re = mag * jnp.cos(ang)
        lb_im = mag * jnp.sin(ang)
        den = lam_re * lam_re + lam_im * lam_im
        nre = lb_re - 1.0
        par_s[0] = lb_re
        par_s[1] = lb_im
        par_s[2] = (nre * lam_re + lb_im * lam_im) / den
        par_s[3] = (lb_im * lam_re - nre * lam_im) / den

    def c_rows(r0, r1):
        co_re, co_im = par_s[2], par_s[3]
        cre = cre_s[r0:r1, :].astype(F32)
        cim = cim_s[r0:r1, :].astype(F32)
        a = 2.0 * (cre * co_re - cim * co_im)
        b = -2.0 * (cre * co_im + cim * co_re)
        cp_s[r0:r1, 0:DM] = a.astype(BF16)
        cp_s[r0:r1, DM:2 * DM] = b.astype(BF16)
        return a[0:8, 0:128]

    def scan_step(s, st, ar, ai, store):
        st = list(st)
        for lt in range(NLT):
            hr, hi = st[lt], st[NLT + lt]
            ur = u_s[lt, pl.ds(s, NCHUNK, stride=CLEN), :]
            ui = u_s[NLT + lt, pl.ds(s, NCHUNK, stride=CLEN), :]
            nr = ar[lt] * hr - ai[lt] * hi + ur
            ni = ar[lt] * hi + ai[lt] * hr + ui
            if store:
                u_s[lt, pl.ds(s, NCHUNK, stride=CLEN), :] = nr
                u_s[NLT + lt, pl.ds(s, NCHUNK, stride=CLEN), :] = ni
            st[lt], st[NLT + lt] = nr, ni
        return tuple(st)

    def chunk_carry(ends, ar, ai):
        row = jax.lax.broadcasted_iota(jnp.int32, (NCHUNK, 128), 0)
        init = []
        for lt in range(NLT):
            br, bi = ar[lt], ai[lt]
            pr = pi = None
            e = CLEN
            while e:
                if e & 1:
                    pr, pi = (br, bi) if pr is None else _cmul(pr, pi, br, bi)
                e >>= 1
                if e:
                    br, bi = _cmul(br, bi, br, bi)
            hr = jnp.where(row >= 1, pltpu.roll(ends[lt], 1, 0), 0.0)
            hi = jnp.where(row >= 1, pltpu.roll(ends[NLT + lt], 1, 0), 0.0)
            sh = 1
            while sh < NCHUNK:
                sr = jnp.where(row >= sh, pltpu.roll(hr, sh, 0), 0.0)
                si = jnp.where(row >= sh, pltpu.roll(hi, sh, 0), 0.0)
                dr, di = _cmul(pr, pi, sr, si)
                hr, hi = hr + dr, hi + di
                pr, pi = _cmul(pr, pi, pr, pi)
                sh *= 2
            init.append((hr, hi))
        return tuple(h[0] for h in init) + tuple(h[1] for h in init)

    class PacedScan:
        def __init__(self, nslices):
            lb_re, lb_im = par_s[0], par_s[1]
            tile = lambda v, lt: jnp.broadcast_to(v[:, lt * 128:(lt + 1) * 128], (NCHUNK, 128))
            self.ar = [tile(lb_re, lt) for lt in range(NLT)]
            self.ai = [tile(lb_im, lt) for lt in range(NLT)]
            self.st = tuple(jnp.zeros((NCHUNK, 128), F32) for _ in range(2 * NLT))
            self.items = [(False, s) for s in range(CLEN)] + [None] + [(True, s) for s in range(CLEN)]
            self.n = nslices
            self.crows = {(k * nslices) // (DM // CROWS): k for k in range(DM // CROWS)}

        def __call__(self, i, hist):
            lo = (i * len(self.items)) // self.n
            hi = ((i + 1) * len(self.items)) // self.n
            if i >= LAG:
                zin = _zero_of(hist[i - LAG])
                self.st = tuple(h + zin for h in self.st[:NLT]) + tuple(self.st[NLT:])
            for it in self.items[lo:hi]:
                if it is None:
                    self.st = chunk_carry(self.st, self.ar, self.ai)
                else:
                    self.st = scan_step(it[1], self.st, self.ar, self.ai, it[0])
            dep = (self.st[0] + self.st[1]) + (self.st[2] + self.st[3])
            if i in self.crows:
                k = self.crows[i]
                dep = dep + c_rows(CROWS * k, CROWS * (k + 1))
            return _zero_of(dep)

    def proj_ssm_half(i, b_s, lt0):
        r0 = pl.multiple_of(i * TQ, TQ)
        u = _dot(xb_s[pl.ds(r0, TQ), :], b_s[...], _NT)
        for lt in range(NLT):
            u_s[lt0 + lt, pl.ds(r0, TQ), :] = u[:, lt * 128:(lt + 1) * 128]

    def proj_ssm_block(i):
        proj_ssm_half(i, bre_s, 0)
        proj_ssm_half(i, bim_s, NLT)

    def proj_attn_block(i):
        r0 = pl.multiple_of(i * TQ, TQ)
        xc = x_s[pl.ds(r0, TQ), :]
        q = _dot(wt_s[0], xc, _NT).astype(BF16)
        qt = (q.astype(F32) * QSCALE).astype(BF16)
        qt_s[i] = qt
        for hq in range(PPB):
            qf_s[i * PPB + hq] = qt[hq * UN * DH:(hq + 1) * UN * DH, :].astype(F32)
        vt_s[i] = _dot(wt_s[1], xc, _NT).astype(BF16)
        k = _dot(xc, w_s[1]).astype(BF16)
        for p in range(NHEAD // KG):
            kp_s[p, pl.ds(r0, TQ), :] = k[:, DH * KG * p:DH * KG * (p + 1)]
        for cc in range(TQ // CK):
            kr = k[(cc + 1) * CK - VR:(cc + 1) * CK, :].astype(F32)
            row = pl.multiple_of((i * (TQ // CK) + cc) * VR, VR)
            for lt in range(NLT):
                kf_s[lt, pl.ds(row, VR), :] = kr[:, lt * 128:(lt + 1) * 128]

    NPAIR = NQB // PU

    @pl.when(j == 0)
    def _prologue():
        copy(S_BRE).start()
        xb_copy(0).start()
        ssm_params()
        copy(S_BIM).start()
        xb_copy(1).start()
        for lt in range(2 * NLT):
            u_s[lt, SEQ:UROWS, :] = jnp.zeros((UROWS - SEQ, 128), F32)
        copy(S_BRE).wait()
        xb_copy(0).wait()
        proj_ssm_half(0, bre_s, 0)
        copy(S_BIM).wait()
        for r in range(PU, NQB):
            xb_copy(r).start()
        proj_ssm_half(0, bim_s, NLT)
        xb_copy(1).wait()
        proj_ssm_block(1)

        def proj_ssm(i, carry):
            for u in range(PU):
                xb_copy(i * PU + u).wait()

            @pl.when(i == 1)
            def _():
                for k in (S_WQ, S_WV, S_WK):
                    copy(k).start()
                for r in range(NQB):
                    x_copy(r).start()

            for u in range(PU):
                proj_ssm_block(i * PU + u)
            return carry
        jax.lax.fori_loop(1, NPAIR - 1, proj_ssm, 0)

        for u in range(PU):
            xb_copy(NQB - PU + u).wait()
        copy(S_WQ).wait()
        copy(S_WV).wait()
        for k in (S_CRE, S_CIM, S_WO):
            copy(k).start()
        for u in range(PU):
            proj_ssm_block(NQB - PU + u)
            wt_s[u] = w_s[2 * u].T
        copy(S_WK).wait()

        def proj_attn(i, carry):
            for u in range(PA):
                x_copy(i * PA + u).wait()
            for u in range(PA):
                proj_attn_block(i * PA + u)
            return carry
        jax.lax.fori_loop(0, NQB // PA, proj_attn, 0)

        for k in (S_CRE, S_CIM, S_WO):
            copy(k).wait()

    @pl.when(j == 0)
    def _fill():
        phase(-1, A, B, do_pv=False, pre_qk=PacedScan(UN * NC))

    nph = jnp.where(j == NQB - 1, PPB - 1, PPB)

    def phase_pair(i, carry):
        ph = j * PPB + 2 * i
        phase(ph, B, A)

        @pl.when(2 * i + 1 < nph)
        def _odd():
            phase(ph + 1, A, B)
        return carry

    jax.lax.fori_loop(0, PPB // 2, phase_pair, 0)

    slot = j % 2

    @pl.when(j >= 2)
    def _free_slot():
        out_copy(j - 2, 0).wait()
        out_copy(j - 2, 1).wait()

    def ssm_out():
        r0 = pl.multiple_of(j * TQ, TQ)
        g = jnp.concatenate([u_s[lt, pl.ds(r0, TQ), :] for lt in range(2 * NLT)], axis=1).astype(BF16)
        y = _dot(g, cp_s[...], _NT)
        d = dsk_ref[...].astype(F32).reshape(1, DM)
        o_s[slot, :, DM:2 * DM] = y + xb_s[pl.ds(r0, TQ), :].astype(F32) * d

    def attn_out():
        o = (ot_s[...] * (1.0 / ls_s[...])).reshape(DM, TQ).astype(BF16)
        o_s[slot, :, 0:DM] = _dot(o, wo_s[...], _TN)

    class SsmOutPieces:
        def __init__(self, nsteps):
            self.r0 = (NQB - 1) * TQ
            self.npieces = NLT * 2 * NLT
            self.at = {(p * nsteps) // self.npieces: p for p in range(self.npieces)}
            self.acc = None

        def __call__(self, i):
            if i not in self.at:
                return
            n, k = divmod(self.at[i], 2 * NLT)
            g = u_s[k, self.r0:self.r0 + TQ, :].astype(BF16)
            part = _dot(g, cp_s[n * 128:(n + 1) * 128, k * 128:(k + 1) * 128], _NT)
            self.acc = part if k == 0 else self.acc + part
            if k == 2 * NLT - 1:
                d = dsk_ref[...].astype(F32).reshape(1, DM)[:, n * 128:(n + 1) * 128]
                xb = xb_s[self.r0:self.r0 + TQ, n * 128:(n + 1) * 128].astype(F32)
                o_s[(NQB - 1) % 2, :, DM + n * 128:DM + (n + 1) * 128] = self.acc + xb * d

    @pl.when(j < NQB - 1)
    def _notlast():
        ssm_out()
        attn_out()
        out_copy(j, 0).start()
        out_copy(j, 1).start()

    @pl.when(j == NQB - 1)
    def _last():
        phase(NPH - 1, A, B, do_qk=False, side=SsmOutPieces(UN * NC))
        out_copy(j, 1).start()

    @pl.when(j == NQB - 1)
    def _last2():
        attn_out()
        out_copy(j, 0).start()
        out_copy(j - 1, 0).wait()
        out_copy(j - 1, 1).wait()
        out_copy(j, 1).wait()
        out_copy(j, 0).wait()


@jax.jit
def pallas_concat_heads__softmax_full_mha__ssm_conv_s5__prompt_kernel(
    A_x, A_wqkv, A_wo, B_x, B_Lambda_re, B_Lambda_im, B_B_re, B_B_im, B_C_re, B_C_im,
    B_log_dt, B_Dskip,
):
    hbm = pl.BlockSpec(memory_space=pl.ANY)
    vec = pl.BlockSpec((DM,), lambda j: (0,))
    args = (A_x.reshape(SEQ, DM), A_wqkv, A_wo, B_x.reshape(SEQ, DM), B_Lambda_re,
            B_Lambda_im, B_B_re, B_B_im, B_C_re, B_C_im, B_log_dt, B_Dskip)
    in_specs = [hbm, hbm, hbm, hbm, vec, vec, hbm, hbm, hbm, hbm, vec, vec]
    scratch = [
        pltpu.VMEM((SEQ, DM), BF16),
        pltpu.VMEM((3, DM, DM), BF16),
        pltpu.VMEM((DM, DM), BF16),
        pltpu.VMEM((SEQ, DM), BF16),
        pltpu.VMEM((DM, DM), BF16),
        pltpu.VMEM((DM, DM), BF16),
        pltpu.VMEM((DM, DM), BF16),
        pltpu.VMEM((DM, DM), BF16),
        pltpu.VMEM((2, TQ, 2 * DM), F32),
        pltpu.SemaphoreType.DMA((NSEM,)),
        pltpu.VMEM((2, DM, DM), BF16),
        pltpu.VMEM((NQB, DM, TQ), BF16),
        pltpu.VMEM((NQB, DM, TQ), BF16),
        pltpu.VMEM((NHEAD // KG, SEQ, DH * KG), BF16),
        pltpu.VMEM((UN, SEQ, TQ), F32),
        pltpu.VMEM((UN, SEQ, TQ), F32),
        pltpu.VMEM((UN, 1, TQ), F32),
        pltpu.VMEM((UN, 1, TQ), F32),
        pltpu.VMEM((NHEAD, DH, TQ), F32),
        pltpu.VMEM((NHEAD, 1, TQ), F32),
        pltpu.VMEM((2 * NLT, UROWS, 128), F32),
        pltpu.VMEM((DM, 2 * DM), BF16),
        pltpu.VMEM((NLT, NC * VR, 128), F32),
        pltpu.VMEM((NPH, UN * DH, TQ), F32),
        pltpu.VMEM((4, 1, DM), F32),
    ]
    out = pl.pallas_call(
        _kernel,
        grid=(NQB,),
        in_specs=in_specs,
        out_specs=pl.BlockSpec(memory_space=pl.ANY),
        out_shape=jax.ShapeDtypeStruct((SEQ, 2 * DM), F32),
        scratch_shapes=scratch,
        compiler_params=pltpu.CompilerParams(
            dimension_semantics=("arbitrary",),
            vmem_limit_bytes=110 * 1024 * 1024),
    )(*args)
    return out.reshape(1, SEQ, 2 * DM)
```
